```python
import jax
import jax.numpy as jnp

def _softmax(x, axis=-1):
    return jax.nn.softmax(x, axis=axis)
def _gelu(x):
    return jax.nn.gelu(x, approximate=True)
def _silu(x):
    return jax.nn.silu(x)
def _sigmoid(x):
    return jax.nn.sigmoid(x)
def _layernorm(x, axis=-1, eps=1e-5):
    m = jnp.mean(x, axis=axis, keepdims=True)
    v = jnp.var(x, axis=axis, keepdims=True)
    return (x - m) / jnp.sqrt(v + eps)
def _scatter_add(tgt, idx, src, axis=0):
    return tgt.at[idx].add(src)
def _segment_sum(src, seg, n):
    return jax.ops.segment_sum(src, seg, n)
class _Rng:
    def __init__(self, key):
        self._k = key
    def _next(self):
        self._k, sub = jax.random.split(self._k)
        return sub
    def normal(self, shape):
        return jax.random.normal(self._next(), shape, dtype=jnp.bfloat16)
    def randint(self, lo, hi, shape):
        return jax.random.randint(self._next(), shape, lo, hi, dtype=jnp.int32)
    def uniform(self, shape, lo=0.0, hi=1.0):
        return jax.random.uniform(self._next(), shape, jnp.bfloat16, lo, hi)
    def permutation(self, n):
        return jax.random.permutation(self._next(), n)


kernel_name = 'concat_heads__compressed_kv_cla__gqa_block_cached__decode'

def setup_inputs():
    _rng = _Rng(jax.random.key(int.from_bytes(__import__("os").urandom(4), "little")))
    _w = (lambda a: (lambda t: t.astype(jnp.bfloat16) if jnp.issubdtype(t.dtype, jnp.floating) else t)(jnp.asarray(a)))
    def _A_setup():
        B, H, Sq, Sk, D, M = 2, 32, 1, 4096, 128, 512
        Dc = 4 * D
        return {
            "x": _w((lambda *s: _rng.normal(s) * 0.05)(B, Sq, M)),
            "c_kv": _w((lambda *s: _rng.normal(s) * 0.05)(B, Sk, Dc)),
            "w_q": _w((lambda *s: _rng.normal(s) * 0.05)(M, H, D) * (M ** -0.5)),
            "w_uk": _w((lambda *s: _rng.normal(s) * 0.05)(Dc, H, D) * (Dc ** -0.5)),
            "w_uv": _w((lambda *s: _rng.normal(s) * 0.05)(Dc, H, D) * (Dc ** -0.5)),
            "w_o": _w((lambda *s: _rng.normal(s) * 0.05)(H, D, M) * ((H * D) ** -0.5)),
        }
    _A_in = _A_setup()

    def _B_setup():
        B, Sq, D = 2, 1, 512
        Hq, Hkv, Sk, Dh = 32, 32, 4096, 128
        assert Hq % Hkv == 0, (Hq, Hkv)
        return {
            "x": _w((lambda *s: _rng.normal(s) * 0.05)(B, Sq, D)),
            "k_cache": _w((lambda *s: _rng.normal(s) * 0.05)(B, Hkv, Sk, Dh)),
            "v_cache": _w((lambda *s: _rng.normal(s) * 0.05)(B, Hkv, Sk, Dh)),
            "wq": _w((lambda *s: _rng.normal(s) * 0.05)(D, Hq * Dh) * (D ** -0.5)),
            "wo": _w((lambda *s: _rng.normal(s) * 0.05)(Hq * Dh, D) * ((Hq * Dh) ** -0.5)),
        }
    _B_in = _B_setup()

    return {
        "A_x": _A_in["x"],
        "A_c_kv": _A_in["c_kv"],
        "A_w_q": _A_in["w_q"],
        "A_w_uk": _A_in["w_uk"],
        "A_w_uv": _A_in["w_uv"],
        "A_w_o": _A_in["w_o"],
        "B_x": _B_in["x"],
        "B_k_cache": _B_in["k_cache"],
        "B_v_cache": _B_in["v_cache"],
        "B_wq": _B_in["wq"],
        "B_wo": _B_in["wo"],
    }

def reference(A_x, A_c_kv, A_w_q, A_w_uk, A_w_uv, A_w_o, B_x, B_k_cache, B_v_cache, B_wq, B_wo):
    def _A_ref(x, c_kv, w_q, w_uk, w_uv, w_o):
        B, Sq, M = x.shape[0], x.shape[1], x.shape[2]
        Sk = c_kv.shape[1]
        H, D = w_q.shape[1], w_q.shape[2]
        q = jnp.einsum("bqm,mhd->bhqd", x, w_q)
        k = jnp.einsum("bkc,chd->bhkd", c_kv, w_uk)
        v = jnp.einsum("bkc,chd->bhkd", c_kv, w_uv)
        scores = jnp.einsum("bhqd,bhkd->bhqk", q, k) * (D ** -0.5)
        off = Sk - Sq
        qi = jnp.arange(Sq)[:, None]
        kj = jnp.arange(Sk)[None, :]
        cmask = kj <= (qi + off)
        scores = jnp.where(cmask[None, None], scores, -1e9)
        p = _softmax(scores, axis=-1)
        ctx = jnp.einsum("bhqk,bhkd->bhqd", p, v)
        return jnp.einsum("bhqd,hdm->bqm", ctx, w_o)

    def _B_ref(x, k_cache, v_cache, wq, wo):
        B, Sq, D = x.shape
        Hq, Dh = 32, 128
        Hkv = k_cache.shape[1]
        rep = Hq // Hkv
        q = (lambda x, *d: x.transpose(*d))((x @ wq).reshape(B, Sq, Hq, Dh), 0, 2, 1, 3)
        k = jnp.repeat(k_cache, rep, axis=1)
        v = jnp.repeat(v_cache, rep, axis=1)
        scores = jnp.einsum("bhqd,bhkd->bhqk", q, k) * (Dh ** -0.5)
        p = _softmax(scores, axis=-1)
        o = jnp.einsum("bhqk,bhkd->bhqd", p, v)
        return (lambda x, *d: x.transpose(*d))(o, 0, 2, 1, 3).reshape(B, Sq, Hq * Dh) @ wo

    a = _A_ref(A_x, A_c_kv, A_w_q, A_w_uk, A_w_uv, A_w_o)
    b = _B_ref(B_x, B_k_cache, B_v_cache, B_wq, B_wo)
    return jnp.concatenate([a, b], axis=-1)
```

```python
import jax
import jax.numpy as jnp
from jax import lax
from jax.experimental import pallas as pl
from jax.experimental.pallas import tpu as pltpu

_B = 2
_H = 32
_D = 128
_M = 512
_S = 4096
_BH = _B * _H

_NSLOT = 8
_A_STEP = _NSLOT
_KC = 512
_WO_HEADS = 8
_WO_CHUNKS = _H // _WO_HEADS

_F32 = jnp.float32
_BF16 = jnp.bfloat16
_NT = (((1,), (1,)), ((), ()))


def _dot(a, b):
    return jnp.dot(a, b, preferred_element_type=_F32)


def _dot_nt(a, b):
    return lax.dot_general(a, b, _NT, preferred_element_type=_F32)


def _iota(shape, dim):
    return lax.broadcasted_iota(jnp.int32, shape, dim)


def _same_head_mask():
    shape = (4 * _BH, 128)
    return (_iota(shape, 0) & (_H - 1)) == (_iota(shape, 1) & (_H - 1))


def _w_rows(w_ref, a, j):
    return w_ref[pl.ds(pl.multiple_of(a * (128 * _H) + j * 128, 128), 128), :]


def _per_head_contract(lhs, w_ref):
    stacked = jnp.concatenate([lhs[:, a * 128:(a + 1) * 128] for a in range(4)], axis=0)
    same_head = _same_head_mask()
    src_minus_cl = _iota((128, 128), 0) - (_iota((128, 128), 1) >> 5)

    def step(j, acc):
        spread = jnp.where(src_minus_cl == 4 * j, 1.0, 0.0).astype(_BF16)
        e = jnp.where(same_head, _dot(stacked, spread), 0.0).astype(_BF16)
        for a in range(4):
            acc = acc + _dot(e[a * _BH:(a + 1) * _BH], _w_rows(w_ref, a, j))
        return acc

    return lax.fori_loop(0, _H, step, jnp.zeros((_BH, _D), _F32))


def _per_head_project(q, w_ref):
    same_head = _same_head_mask()
    dst_minus_cl = _iota((128, 128), 1) - (_iota((128, 128), 0) >> 5)

    def step(j, acc):
        t = jnp.concatenate([_dot_nt(q, _w_rows(w_ref, a, j)) for a in range(4)], axis=0)
        t = jnp.where(same_head, t, 0.0).astype(_BF16)
        gather = jnp.where(dst_minus_cl == 4 * j, 1.0, 0.0).astype(_BF16)
        return acc + _dot(t, gather)

    acc = lax.fori_loop(0, _H, step, jnp.zeros((4 * _BH, 128), _F32))
    return jnp.concatenate([acc[a * _BH:(a + 1) * _BH] for a in range(4)], axis=1)


def _latent_attention(qa, ckv_ref, s_ref):
    scale = _D ** -0.5

    def keys(t):
        return ckv_ref[pl.ds(pl.multiple_of(t * _KC, _KC), _KC), :]

    def scores(t, m):
        s = _dot_nt(qa, keys(t)) * scale
        s_ref[t] = s
        return jnp.maximum(m, s)

    m = lax.fori_loop(0, _S // _KC, scores, jnp.full((_H, _KC), -jnp.inf, _F32))
    m = jnp.max(m, axis=1, keepdims=True)

    def values(t, carry):
        l, acc = carry
        p = jnp.exp(s_ref[t] - m)
        return l + p, acc + _dot(p.astype(_BF16), keys(t))

    l, acc = lax.fori_loop(0, _S // _KC, values,
                           (jnp.zeros((_H, _KC), _F32), jnp.zeros((_H, _M), _F32)))
    return acc / jnp.sum(l, axis=1, keepdims=True)


def _out_proj_chunk(ctx_ref, w_ref, g):
    heads = [ctx_ref[pl.ds(g * _WO_HEADS + i, _B, stride=_H), :] for i in range(_WO_HEADS)]
    flat = jnp.concatenate(heads, axis=1).astype(_BF16)
    rows = _WO_HEADS * _D
    return _dot(flat, w_ref[pl.ds(g * rows, rows), :])


def _kernel(ax_hbm, ckv_hbm, awq_hbm, awuk_hbm, awuv_hbm, awo_hbm,
            bx_hbm, k_hbm, v_hbm, bwq_hbm, bwo_hbm,
            out_ref,
            ax_v, bx_v, ckv_v, awq_v, awuk_v, awuv_v, awo_v, bwq_v, bwo_v, k_v, v_v,
            qb_s, ob_s, ctx_s, s_s,
            sem_in, sem_ckv, sem_k, sem_v, sem_awo, sem_bwo):
    cp_bwq = pltpu.make_async_copy(bwq_hbm, bwq_v, sem_in.at[0])
    cp_bx = pltpu.make_async_copy(bx_hbm, bx_v, sem_in.at[1])
    cp_ax = pltpu.make_async_copy(ax_hbm, ax_v, sem_in.at[2])
    cp_awq = pltpu.make_async_copy(awq_hbm, awq_v, sem_in.at[3])
    cp_awuk = pltpu.make_async_copy(awuk_hbm, awuk_v, sem_in.at[4])
    cp_awuv = pltpu.make_async_copy(awuv_hbm, awuv_v, sem_in.at[5])
    cp_ckv = [pltpu.make_async_copy(ckv_hbm.at[b], ckv_v.at[b], sem_ckv.at[b])
              for b in range(_B)]

    def wo_copies(hbm, vmem, sem):
        rows = _WO_HEADS * _D
        return [pltpu.make_async_copy(hbm.at[pl.ds(g * rows, rows)],
                                      vmem.at[pl.ds(g * rows, rows)], sem.at[g])
                for g in range(_WO_CHUNKS)]

    cp_awo = wo_copies(awo_hbm, awo_v, sem_awo)
    cp_bwo = wo_copies(bwo_hbm, bwo_v, sem_bwo)

    def cp_k(i, slot):
        return pltpu.make_async_copy(k_hbm.at[i], k_v.at[slot], sem_k.at[slot])

    def cp_v(i, slot):
        return pltpu.make_async_copy(v_hbm.at[i], v_v.at[slot], sem_v.at[slot])

    cp_bwq.start()
    cp_bx.start()
    cp_ax.start()
    for i in range(_NSLOT):
        cp_k(i, i).start()
        cp_v(i, i).start()
    cp_awq.start()
    cp_awuk.start()
    for cp in cp_ckv:
        cp.start()
    cp_awuv.start()

    cp_bx.wait()
    cp_bwq.wait()
    qb = _dot(bx_v[...], bwq_v[...])
    for h in range(_H):
        qb_s[pl.ds(h, _B, stride=_H), :] = qb[:, h * _D:(h + 1) * _D]

    def branch_a():
        cp_ax.wait()
        x = ax_v[...].astype(_F32)
        x_rows = jnp.concatenate(
            [jnp.broadcast_to(x[b:b + 1], (_H, _M)) for b in range(_B)], axis=0)
        cp_awq.wait()
        q = _per_head_contract(x_rows.astype(_BF16), awq_v)
        cp_awuk.wait()
        qa = _per_head_project(q.astype(_BF16), awuk_v).astype(_BF16)
        latent = []
        for b in range(_B):
            cp_ckv[b].wait()
            latent.append(_latent_attention(qa[b * _H:(b + 1) * _H], ckv_v.at[b], s_s))
        cp_awuv.wait()
        ctx_s[...] = _per_head_contract(
            jnp.concatenate(latent, axis=0).astype(_BF16), awuv_v)

    def head(i, carry):
        pl.when(i == _A_STEP)(branch_a)

        slot = i % _NSLOT
        q = jnp.broadcast_to(qb_s[pl.ds(i, 1), :], (8, _D)).astype(_BF16)
        cp_k(i, slot).wait()
        s = _dot_nt(q, k_v[slot]) * (_D ** -0.5)
        p = jnp.exp(s - jnp.max(s, axis=1, keepdims=True))
        l = jnp.sum(p, axis=1, keepdims=True)
        cp_v(i, slot).wait()
        o = _dot(p.astype(_BF16), v_v[slot]) / l
        ob_s[pl.ds(i, 1), :] = o[0:1]

        @pl.when(i + _NSLOT < _BH)
        def _():
            cp_k(i + _NSLOT, slot).start()
            cp_v(i + _NSLOT, slot).start()

        @pl.when(i + _NSLOT == _BH)
        def _():
            for cp in cp_awo + cp_bwo:
                cp.start()

        return carry

    lax.fori_loop(0, _BH, head, 0)

    for col, ctx_ref, w_ref, cps in ((0, ctx_s, awo_v, cp_awo), (_M, ob_s, bwo_v, cp_bwo)):
        acc = jnp.zeros((_B, _M), _F32)
        for g in range(_WO_CHUNKS):
            cps[g].wait()
            acc = acc + _out_proj_chunk(ctx_ref, w_ref, g)
        out_ref[:, col:col + _M] = acc.astype(out_ref.dtype)


@jax.jit
def pallas_concat_heads__compressed_kv_cla__gqa_block_cached__decode_kernel(
    A_x: jax.Array,
    A_c_kv: jax.Array,
    A_w_q: jax.Array,
    A_w_uk: jax.Array,
    A_w_uv: jax.Array,
    A_w_o: jax.Array,
    B_x: jax.Array,
    B_k_cache: jax.Array,
    B_v_cache: jax.Array,
    B_wq: jax.Array,
    B_wo: jax.Array,
):
    assert A_x.shape == (_B, 1, _M) and B_x.shape == (_B, 1, _M)
    assert A_c_kv.shape == (_B, _S, _M)
    assert A_w_q.shape == A_w_uk.shape == A_w_uv.shape == (_M, _H, _D)
    assert A_w_o.shape == (_H, _D, _M)
    assert B_k_cache.shape == B_v_cache.shape == (_B, _H, _S, _D)
    assert B_wq.shape == (_M, _H * _D) and B_wo.shape == (_H * _D, _M)

    vmem = pltpu.VMEM
    dma = pltpu.SemaphoreType.DMA
    out = pl.pallas_call(
        _kernel,
        in_specs=[pl.BlockSpec(memory_space=pltpu.HBM)] * 11,
        out_specs=pl.BlockSpec(memory_space=vmem),
        out_shape=jax.ShapeDtypeStruct((_B, 2 * _M), A_x.dtype),
        scratch_shapes=[
            vmem((_B, _M), _BF16),
            vmem((_B, _M), _BF16),
            vmem((_B, _S, _M), _BF16),
            vmem((_M * _H, _D), _BF16),
            vmem((_M * _H, _D), _BF16),
            vmem((_M * _H, _D), _BF16),
            vmem((_H * _D, _M), _BF16),
            vmem((_M, _H * _D), _BF16),
            vmem((_H * _D, _M), _BF16),
            vmem((_NSLOT, _S, _D), _BF16),
            vmem((_NSLOT, _S, _D), _BF16),
            vmem((_BH, _D), _F32),
            vmem((_BH, _D), _F32),
            vmem((_BH, _D), _F32),
            vmem((_S // _KC, _H, _KC), _F32),
            dma((6,)), dma((_B,)), dma((_NSLOT,)), dma((_NSLOT,)),
            dma((_WO_CHUNKS,)), dma((_WO_CHUNKS,)),
        ],
        compiler_params=pltpu.CompilerParams(vmem_limit_bytes=100 * 2**20),
    )(
        A_x.reshape(_B, _M),
        A_c_kv,
        A_w_q.reshape(_M * _H, _D),
        A_w_uk.reshape(_M * _H, _D),
        A_w_uv.reshape(_M * _H, _D),
        A_w_o.reshape(_H * _D, _M),
        B_x.reshape(_B, _M),
        B_k_cache.reshape(_BH, _S, _D),
        B_v_cache.reshape(_BH, _S, _D),
        B_wq,
        B_wo,
    )
    return out.reshape(_B, 1, 2 * _M)
```

```python
import functools

import jax
import jax.numpy as jnp
from jax import lax
from jax.experimental import pallas as pl
from jax.experimental.pallas import tpu as pltpu

_B = 2
_H = 32
_D = 128
_M = 512
_S = 4096
_BH = _B * _H

_NSLOT = 6
_A_GAP = 4
_KC = 512
_V_PRIORITY = 1
_WO_HEADS = (16, 8, 4, 3, 1)
_WO_START = tuple(sum(_WO_HEADS[:g]) for g in range(len(_WO_HEADS)))

_F32 = jnp.float32
_BF16 = jnp.bfloat16
_NT = (((1,), (1,)), ((), ()))


def _dot(a, b):
    return jnp.dot(a, b, preferred_element_type=_F32)


def _dot_nt(a, b):
    return lax.dot_general(a, b, _NT, preferred_element_type=_F32)


def _iota(shape, dim):
    return lax.broadcasted_iota(jnp.int32, shape, dim)


def _same_head_mask():
    shape = (4 * _BH, 128)
    return (_iota(shape, 0) & (_H - 1)) == (_iota(shape, 1) & (_H - 1))


def _w_rows(w_ref, a, j):
    return w_ref[pl.ds(pl.multiple_of(a * (128 * _H) + j * 128, 128), 128), :]


def _per_head_contract(lhs, w_ref):
    stacked = jnp.concatenate([lhs[:, a * 128:(a + 1) * 128] for a in range(4)], axis=0)
    same_head = _same_head_mask()
    src_minus_cl = _iota((128, 128), 0) - (_iota((128, 128), 1) >> 5)

    def step(j, acc):
        spread = jnp.where(src_minus_cl == 4 * j, 1.0, 0.0).astype(_BF16)
        e = jnp.where(same_head, _dot(stacked, spread), 0.0).astype(_BF16)
        for a in range(4):
            acc = acc + _dot(e[a * _BH:(a + 1) * _BH], _w_rows(w_ref, a, j))
        return acc

    return lax.fori_loop(0, _H, step, jnp.zeros((_BH, _D), _F32))


def _per_head_project(q, w_ref):
    same_head = _same_head_mask()
    dst_minus_cl = _iota((128, 128), 1) - (_iota((128, 128), 0) >> 5)

    def step(j, acc):
        t = jnp.concatenate([_dot_nt(q, _w_rows(w_ref, a, j)) for a in range(4)], axis=0)
        t = jnp.where(same_head, t, 0.0).astype(_BF16)
        gather = jnp.where(dst_minus_cl == 4 * j, 1.0, 0.0).astype(_BF16)
        return acc + _dot(t, gather)

    acc = lax.fori_loop(0, _H, step, jnp.zeros((4 * _BH, 128), _F32))
    return jnp.concatenate([acc[a * _BH:(a + 1) * _BH] for a in range(4)], axis=1)


def _latent_attention(qa, ckv_ref, s_ref):
    scale = _D ** -0.5

    def keys(t):
        return ckv_ref[pl.ds(pl.multiple_of(t * _KC, _KC), _KC), :]

    def scores(t, m):
        s = _dot_nt(qa, keys(t)) * scale
        s_ref[t] = s
        return jnp.maximum(m, s)

    m = lax.fori_loop(0, _S // _KC, scores, jnp.full((_H, _KC), -jnp.inf, _F32))
    m = jnp.max(m, axis=1, keepdims=True)

    def values(t, carry):
        l, acc = carry
        p = jnp.exp(s_ref[t] - m)
        return l + p, acc + _dot(p.astype(_BF16), keys(t))

    l, acc = lax.fori_loop(0, _S // _KC, values,
                           (jnp.zeros((_H, _KC), _F32), jnp.zeros((_H, _M), _F32)))
    return acc / jnp.sum(l, axis=1, keepdims=True)


def _out_proj(ctx_ref, w_ref, h0, nh):
    heads = [ctx_ref[pl.ds(h, _B, stride=_H), :] for h in range(h0, h0 + nh)]
    flat = jnp.concatenate(heads, axis=1).astype(_BF16)
    return _dot(flat, w_ref[pl.ds(h0 * _D, nh * _D), :])


def _kernel(ax_hbm, ckv_hbm, awq_hbm, awuk_hbm, awuv_hbm, awo_hbm,
            bx_hbm, k_hbm, v_hbm, bwq_hbm, bwo_hbm,
            out_ref,
            ax_v, bx_v, ckv_v, awq_v, awuk_v, awuv_v, awo_v, bwq_v, bwo_v, k_v, v_v,
            qb_s, ob_s, q_s, qa_s, lat_s, ctx_s, s_s,
            sem_in, sem_ckv, sem_k, sem_v, sem_bwo):
    cp_bx = pltpu.make_async_copy(bx_hbm, bx_v, sem_in.at[0])
    cp_bwq = pltpu.make_async_copy(bwq_hbm, bwq_v, sem_in.at[1])
    cp_ax = pltpu.make_async_copy(ax_hbm, ax_v, sem_in.at[2])
    cp_awq = pltpu.make_async_copy(awq_hbm, awq_v, sem_in.at[3])
    cp_awuk = pltpu.make_async_copy(awuk_hbm, awuk_v, sem_in.at[4])
    cp_awuv = pltpu.make_async_copy(awuv_hbm, awuv_v, sem_in.at[5])
    cp_awo = pltpu.make_async_copy(awo_hbm, awo_v, sem_in.at[6])

    def cp_ckv(b):
        return pltpu.make_async_copy(ckv_hbm.at[b], ckv_v.at[b], sem_ckv.at[b])

    def cp_bwo(g):
        rows = pl.ds(_WO_START[g] * _D, _WO_HEADS[g] * _D)
        return pltpu.make_async_copy(bwo_hbm.at[rows], bwo_v.at[rows], sem_bwo.at[g])

    def cp_k(i, slot):
        return pltpu.make_async_copy(k_hbm.at[i], k_v.at[slot], sem_k.at[slot])

    def cp_v(i, slot):
        return pltpu.make_async_copy(v_hbm.at[i], v_v.at[slot], sem_v.at[slot])

    def start_kv(i, slot):
        cp_k(i, slot).start()
        cp_v(i, slot).start(priority=_V_PRIORITY)

    cp_bwq.start()
    cp_bx.start()
    cp_ax.start()
    lax.fori_loop(0, _NSLOT, lambda i, _: start_kv(i, i), None)

    cp_bx.wait()
    cp_bwq.wait()
    qb = _dot(bx_v[...], bwq_v[...])
    for h in range(_H):
        qb_s[pl.ds(h, _B, stride=_H), :] = qb[:, h * _D:(h + 1) * _D]

    def a_query():
        cp_ax.wait()
        cp_awq.wait()
        x = ax_v[...].astype(_F32)
        x_rows = jnp.concatenate(
            [jnp.broadcast_to(x[b:b + 1], (_H, _M)) for b in range(_B)], axis=0)
        q_s[...] = _per_head_contract(x_rows.astype(_BF16), awq_v).astype(_BF16)

    def a_absorb():
        cp_awuk.wait()
        qa = _per_head_project(q_s[...], awuk_v).astype(_BF16)
        for b in range(_B):
            qa_s[b] = qa[b * _H:(b + 1) * _H]

    def a_attend(b):
        cp_ckv(b).wait()
        lat_s[b] = _latent_attention(qa_s[b], ckv_v.at[b], s_s).astype(_BF16)

    def a_values():
        cp_awuv.wait()
        lat = jnp.concatenate([lat_s[b] for b in range(_B)], axis=0)
        ctx_s[...] = _per_head_contract(lat, awuv_v)

    def a_output():
        cp_awo.wait()
        out_ref[:, :_M] = _out_proj(ctx_s, awo_v, 0, _H).astype(out_ref.dtype)

    def head(i, carry):
        stage = i - (_NSLOT + 1)
        pl.when(stage == 0)(a_query)
        pl.when(stage == _A_GAP)(a_absorb)
        pl.when(jnp.logical_or(stage == 2 * _A_GAP, stage == 3 * _A_GAP))(
            lambda: a_attend((stage == 3 * _A_GAP).astype(jnp.int32)))
        pl.when(stage == 4 * _A_GAP)(a_values)
        pl.when(stage == 5 * _A_GAP)(a_output)

        slot = i % _NSLOT
        q = jnp.broadcast_to(qb_s[pl.ds(i, 1), :], (8, _D)).astype(_BF16)
        cp_k(i, slot).wait()
        s = _dot_nt(q, k_v[slot]) * (_D ** -0.5)
        p = jnp.exp(s - jnp.max(s, axis=1, keepdims=True))
        l = jnp.sum(p, axis=1, keepdims=True)
        cp_v(i, slot).wait()
        o = _dot(p.astype(_BF16), v_v[slot]) / l
        ob_s[pl.ds(i, 1), :] = o[0:1]

        pl.when(i + _NSLOT < _BH)(lambda: start_kv(i + _NSLOT, slot))
        for n, cp in enumerate((cp_awq, cp_awuk, cp_ckv(0), cp_ckv(1), cp_awuv, cp_awo)):
            pl.when(i == n * _A_GAP)(functools.partial(cp.start, priority=_V_PRIORITY))
        for g in range(len(_WO_HEADS)):
            pl.when(i + _NSLOT == _BH + g)(
                functools.partial(cp_bwo(g).start, priority=_V_PRIORITY))
        return carry

    lax.fori_loop(0, _BH, head, 0)

    acc = jnp.zeros((_B, _M), _F32)
    for g in range(len(_WO_HEADS)):
        cp_bwo(g).wait()
        acc = acc + _out_proj(ob_s, bwo_v, _WO_START[g], _WO_HEADS[g])
    out_ref[:, _M:] = acc.astype(out_ref.dtype)


@jax.jit
def pallas_concat_heads__compressed_kv_cla__gqa_block_cached__decode_kernel(
    A_x: jax.Array,
    A_c_kv: jax.Array,
    A_w_q: jax.Array,
    A_w_uk: jax.Array,
    A_w_uv: jax.Array,
    A_w_o: jax.Array,
    B_x: jax.Array,
    B_k_cache: jax.Array,
    B_v_cache: jax.Array,
    B_wq: jax.Array,
    B_wo: jax.Array,
):
    assert A_x.shape == (_B, 1, _M) and B_x.shape == (_B, 1, _M)
    assert A_c_kv.shape == (_B, _S, _M)
    assert A_w_q.shape == A_w_uk.shape == A_w_uv.shape == (_M, _H, _D)
    assert A_w_o.shape == (_H, _D, _M)
    assert B_k_cache.shape == B_v_cache.shape == (_B, _H, _S, _D)
    assert B_wq.shape == (_M, _H * _D) and B_wo.shape == (_H * _D, _M)

    vmem = pltpu.VMEM
    dma = pltpu.SemaphoreType.DMA
    out = pl.pallas_call(
        _kernel,
        in_specs=[pl.BlockSpec(memory_space=pltpu.HBM)] * 11,
        out_specs=pl.BlockSpec(memory_space=vmem),
        out_shape=jax.ShapeDtypeStruct((_B, 2 * _M), A_x.dtype),
        scratch_shapes=[
            vmem((_B, _M), _BF16),
            vmem((_B, _M), _BF16),
            vmem((_B, _S, _M), _BF16),
            vmem((_M * _H, _D), _BF16),
            vmem((_M * _H, _D), _BF16),
            vmem((_M * _H, _D), _BF16),
            vmem((_H * _D, _M), _BF16),
            vmem((_M, _H * _D), _BF16),
            vmem((_H * _D, _M), _BF16),
            vmem((_NSLOT, _S, _D), _BF16),
            vmem((_NSLOT, _S, _D), _BF16),
            vmem((_BH, _D), _F32),
            vmem((_BH, _D), _F32),
            vmem((_BH, _D), _BF16),
            vmem((_B, _H, _M), _BF16),
            vmem((_B, _H, _M), _BF16),
            vmem((_BH, _D), _F32),
            vmem((_S // _KC, _H, _KC), _F32),
            dma((7,)), dma((_B,)), dma((_NSLOT,)), dma((_NSLOT,)), dma((len(_WO_HEADS),)),
        ],
        compiler_params=pltpu.CompilerParams(vmem_limit_bytes=100 * 2**20),
    )(
        A_x.reshape(_B, _M),
        A_c_kv,
        A_w_q.reshape(_M * _H, _D),
        A_w_uk.reshape(_M * _H, _D),
        A_w_uv.reshape(_M * _H, _D),
        A_w_o.reshape(_H * _D, _M),
        B_x.reshape(_B, _M),
        B_k_cache.reshape(_BH, _S, _D),
        B_v_cache.reshape(_BH, _S, _D),
        B_wq,
        B_wo,
    )
    return out.reshape(_B, 1, 2 * _M)
```

```python
import jax
import jax.numpy as jnp
from jax import lax
from jax.experimental import pallas as pl
from jax.experimental.pallas import tpu as pltpu

_B = 2
_H = 32
_D = 128
_M = 512
_S = 4096
_BH = _B * _H

_NSLOT = 3
_PHASE = 8
_PIECE = 16384
_UNROLL = 4
_KC = 512
_WO_HEADS = (16, 8, 4, 3, 1)
_WO_START = tuple(sum(_WO_HEADS[:g]) for g in range(len(_WO_HEADS)))

_F32 = jnp.float32
_BF16 = jnp.bfloat16
_NT = (((1,), (1,)), ((), ()))


def _dot(a, b):
    return jnp.dot(a, b, preferred_element_type=_F32)


def _dot_nt(a, b):
    return lax.dot_general(a, b, _NT, preferred_element_type=_F32)


def _iota(shape, dim):
    return lax.broadcasted_iota(jnp.int32, shape, dim)


def _ds(index, size):
    start = index * size
    return pl.ds(start if isinstance(start, int) else pl.multiple_of(start, size), size)


def _piece(ref, n):
    rows, cols = ref.shape
    if cols * 16 <= _PIECE:
        return ref.at[_ds(n, _PIECE // cols)]
    per_row = cols * 16 // _PIECE
    return ref.at[_ds(n // per_row, 16), _ds(n % per_row, _PIECE // 16)]


def _start_two(src0, dst0, sem0, src1, dst1, sem1):
    def pair(n, _):
        pltpu.make_async_copy(_piece(src0, n), _piece(dst0, n), sem0).start(priority=0)
        pltpu.make_async_copy(_piece(src1, n), _piece(dst1, n), sem1).start(priority=1)
    count = src0.shape[0] * src0.shape[1] // _PIECE
    lax.fori_loop(0, count, pair, None, unroll=min(_UNROLL, count))


def _start_part(src, dst, sem, first, count):
    def pair(j, _):
        for priority in range(2):
            n = 2 * (first + j) + priority
            pltpu.make_async_copy(_piece(src, n), _piece(dst, n), sem).start(priority=priority)
    lax.fori_loop(0, count, pair, None, unroll=min(_UNROLL, count))


def _wait_filled(dst, sem):
    pltpu.make_async_copy(dst, dst, sem).wait()


def _same_head_mask():
    shape = (4 * _BH, 128)
    return (_iota(shape, 0) & (_H - 1)) == (_iota(shape, 1) & (_H - 1))


def _w_rows(w_ref, a, j):
    return w_ref[_ds(a * _H + j, 128), :]


def _stack_columns(x):
    return jnp.concatenate([x[:, a * 128:(a + 1) * 128] for a in range(4)], axis=0)


def _contract_step(j, acc, lhs, w_ref):
    src_minus_cl = _iota((128, 128), 0) - (_iota((128, 128), 1) >> 5)
    spread = jnp.where(src_minus_cl == 4 * j, 1.0, 0.0).astype(_BF16)
    e = jnp.where(_same_head_mask(), _dot(lhs, spread), 0.0).astype(_BF16)
    for a in range(4):
        acc = acc + _dot(e[a * _BH:(a + 1) * _BH], _w_rows(w_ref, a, j))
    return acc


def _project_step(j, acc, q, w_ref):
    t = jnp.concatenate([_dot_nt(q, _w_rows(w_ref, a, j)) for a in range(4)], axis=0)
    t = jnp.where(_same_head_mask(), t, 0.0).astype(_BF16)
    dst_minus_cl = _iota((128, 128), 1) - (_iota((128, 128), 0) >> 5)
    gather = jnp.where(dst_minus_cl == 4 * j, 1.0, 0.0).astype(_BF16)
    return acc + _dot(t, gather)


def _out_proj(ctx_ref, w_ref, h0, nh):
    heads = [ctx_ref[pl.ds(h, _B, stride=_H), :] for h in range(h0, h0 + nh)]
    flat = jnp.concatenate(heads, axis=1).astype(_BF16)
    return _dot(flat, w_ref[pl.ds(h0 * _D, nh * _D), :])


def _kernel(ax_hbm, ckv_hbm, awq_hbm, awuk_hbm, awuv_hbm, awo_hbm,
            bx_hbm, k_hbm, v_hbm, bwq_hbm, bwo_hbm,
            out_ref,
            ax_v, bx_v, ckv_v, awq_v, awuk_v, awuv_v, awo_v, bwq_v, bwo_v, k_v, v_v,
            qb_s, ob_s, lhs_s, acc_s, qa_acc_s, qa_s, s_s, m_s, l_s, lat_s,
            sem_in, sem_ckv, sem_k, sem_v, sem_bwo):
    scale = _D ** -0.5
    cp_ax = pltpu.make_async_copy(ax_hbm, ax_v, sem_in.at[0])
    cp_bx = pltpu.make_async_copy(bx_hbm, bx_v, sem_in.at[1])
    sem_bwq, sem_awq, sem_awuk, sem_awuv, sem_awo = (sem_in.at[n] for n in range(2, 7))
    weight_pairs = _M * _H * _D // _PIECE // 2

    def start_kv(i, slot):
        _start_two(k_hbm.at[i], k_v.at[slot], sem_k.at[slot],
                   v_hbm.at[i], v_v.at[slot], sem_v.at[slot])

    cp_bx.start()
    cp_ax.start()
    _start_part(bwq_hbm, bwq_v, sem_bwq, 0, weight_pairs)
    start_kv(0, 0)

    cp_bx.wait()
    _wait_filled(bwq_v, sem_bwq)
    qb = _dot(bx_v[...], bwq_v[...])
    for h in range(_H):
        qb_s[pl.ds(h, _B, stride=_H), :] = qb[:, h * _D:(h + 1) * _D]
    lax.fori_loop(1, _NSLOT, lambda i, _: start_kv(i, i), None)

    def fetch(src, dst, sem, t):
        _start_part(src, dst, sem, t * (weight_pairs // _PHASE), weight_pairs // _PHASE)

    def contract(w_ref, t):
        n = _H // _PHASE
        lhs = lhs_s[...]
        acc_s[...] = lax.fori_loop(
            t * n, (t + 1) * n, lambda j, acc: _contract_step(j, acc, lhs, w_ref), acc_s[...])

    def a_query(t):
        @pl.when(t == 0)
        def _():
            cp_ax.wait()
            _wait_filled(awq_v, sem_awq)
            x = ax_v[...].astype(_F32)
            x_rows = jnp.concatenate(
                [jnp.broadcast_to(x[b:b + 1], (_H, _M)) for b in range(_B)], axis=0)
            lhs_s[...] = _stack_columns(x_rows).astype(_BF16)
            acc_s[...] = jnp.zeros(acc_s.shape, _F32)

        contract(awq_v, t)

    def a_absorb(t):
        @pl.when(t == 0)
        def _():
            _wait_filled(awuk_v, sem_awuk)
            qa_acc_s[...] = jnp.zeros(qa_acc_s.shape, _F32)

        n = _H // _PHASE
        q = acc_s[...].astype(_BF16)
        qa_acc_s[...] = lax.fori_loop(
            t * n, (t + 1) * n, lambda j, acc: _project_step(j, acc, q, awuk_v), qa_acc_s[...])

        @pl.when(t == _PHASE - 1)
        def _():
            for b in range(_B):
                qa_s[b] = jnp.concatenate(
                    [qa_acc_s[pl.ds(a * _BH + b * _H, _H), :] for a in range(4)],
                    axis=1).astype(_BF16)

    def a_attend(b, t):
        half = _PHASE // 2
        n = _S // _KC // half

        @pl.when(t == 0)
        def _():
            _wait_filled(ckv_v.at[b], sem_ckv.at[b])
            m_s[...] = jnp.full(m_s.shape, -jnp.inf, _F32)

        @pl.when(t < half)
        def _():
            qa = qa_s[b]

            def scores(c, m):
                s = _dot_nt(qa, ckv_v[b, _ds(c, _KC), :]) * scale
                s_s[c] = s
                return jnp.maximum(m, s)

            m_s[...] = lax.fori_loop(t * n, (t + 1) * n, scores, m_s[...])

        @pl.when(t == half)
        def _():
            m_s[...] = jnp.broadcast_to(jnp.max(m_s[...], axis=1, keepdims=True), m_s.shape)
            l_s[...] = jnp.zeros(l_s.shape, _F32)
            lat_s[b] = jnp.zeros((_H, _M), _F32)

        @pl.when(t >= half)
        def _():
            m = m_s[...]

            def values(c, carry):
                l, acc = carry
                p = jnp.exp(s_s[c] - m)
                return l + p, acc + _dot(p.astype(_BF16), ckv_v[b, _ds(c, _KC), :])

            l_s[...], lat_s[b] = lax.fori_loop(
                (t - half) * n, (t - half + 1) * n, values, (l_s[...], lat_s[b]))

        @pl.when(t == _PHASE - 1)
        def _():
            lat_s[b] = lat_s[b] / jnp.sum(l_s[...], axis=1, keepdims=True)

    def a_values(t):
        @pl.when(t == 0)
        def _():
            _wait_filled(awuv_v, sem_awuv)
            lat = jnp.concatenate([lat_s[b] for b in range(_B)], axis=0)
            lhs_s[...] = _stack_columns(lat).astype(_BF16)
            acc_s[...] = jnp.zeros(acc_s.shape, _F32)

        contract(awuv_v, t)

    def a_output():
        _wait_filled(awo_v, sem_awo)
        out_ref[:, :_M] = _out_proj(acc_s, awo_v, 0, _H).astype(out_ref.dtype)

    def step(i, carry):
        slot = i % _NSLOT
        q = jnp.broadcast_to(qb_s[pl.ds(i, 1), :], (8, _D)).astype(_BF16)
        _wait_filled(k_v.at[slot], sem_k.at[slot])
        s = _dot_nt(q, k_v[slot]) * scale
        p = jnp.exp(s - jnp.max(s, axis=1, keepdims=True))
        l = jnp.sum(p, axis=1, keepdims=True)
        _wait_filled(v_v.at[slot], sem_v.at[slot])
        o = _dot(p.astype(_BF16), v_v[slot]) / l
        ob_s[pl.ds(i, 1), :] = o[0:1]

        pl.when(i + _NSLOT < _BH)(lambda: start_kv(i + _NSLOT, slot))

        pairs_per_head = _D * _M // _PIECE // 2
        for g in range(len(_WO_HEADS)):
            pl.when(i + _NSLOT == _BH + min(g, _NSLOT - 1))(
                lambda g=g: _start_part(bwo_hbm, bwo_v, sem_bwo.at[g],
                                        _WO_START[g] * pairs_per_head,
                                        _WO_HEADS[g] * pairs_per_head))

        phase, t = i // _PHASE, i % _PHASE

        @pl.when(phase == 0)
        def _():
            fetch(awq_hbm, awq_v, sem_awq, t)

        @pl.when(phase == 1)
        def _():
            a_query(t)
            fetch(awuk_hbm, awuk_v, sem_awuk, t)

        @pl.when(phase == 2)
        def _():
            a_absorb(t)

        @pl.when(jnp.logical_or(phase == 3, phase == 4))
        def _():
            a_attend(phase - 3, t)

        @pl.when(jnp.logical_or(phase == 2, phase == 3))
        def _():
            fetch(ckv_hbm.at[phase - 2], ckv_v.at[phase - 2], sem_ckv.at[phase - 2], t)

        @pl.when(phase == 4)
        def _():
            fetch(awuv_hbm, awuv_v, sem_awuv, t)

        @pl.when(phase == 5)
        def _():
            a_values(t)
            fetch(awo_hbm, awo_v, sem_awo, t)

        pl.when(i == 6 * _PHASE)(a_output)
        return carry

    lax.fori_loop(0, _BH, step, 0)

    acc = jnp.zeros((_B, _M), _F32)
    for g in range(len(_WO_HEADS)):
        _wait_filled(bwo_v.at[pl.ds(_WO_START[g] * _D, _WO_HEADS[g] * _D)], sem_bwo.at[g])
        acc = acc + _out_proj(ob_s, bwo_v, _WO_START[g], _WO_HEADS[g])
    out_ref[:, _M:] = acc.astype(out_ref.dtype)


@jax.jit
def pallas_concat_heads__compressed_kv_cla__gqa_block_cached__decode_kernel(
    A_x: jax.Array,
    A_c_kv: jax.Array,
    A_w_q: jax.Array,
    A_w_uk: jax.Array,
    A_w_uv: jax.Array,
    A_w_o: jax.Array,
    B_x: jax.Array,
    B_k_cache: jax.Array,
    B_v_cache: jax.Array,
    B_wq: jax.Array,
    B_wo: jax.Array,
):
    assert A_x.shape == (_B, 1, _M) and B_x.shape == (_B, 1, _M)
    assert A_c_kv.shape == (_B, _S, _M)
    assert A_w_q.shape == A_w_uk.shape == A_w_uv.shape == (_M, _H, _D)
    assert A_w_o.shape == (_H, _D, _M)
    assert B_k_cache.shape == B_v_cache.shape == (_B, _H, _S, _D)
    assert B_wq.shape == (_M, _H * _D) and B_wo.shape == (_H * _D, _M)

    vmem = pltpu.VMEM
    dma = pltpu.SemaphoreType.DMA
    out = pl.pallas_call(
        _kernel,
        in_specs=[pl.BlockSpec(memory_space=pltpu.HBM)] * 11,
        out_specs=pl.BlockSpec(memory_space=vmem),
        out_shape=jax.ShapeDtypeStruct((_B, 2 * _M), A_x.dtype),
        scratch_shapes=[
            vmem((_B, _M), _BF16),
            vmem((_B, _M), _BF16),
            vmem((_B, _S, _M), _BF16),
            vmem((_M * _H, _D), _BF16),
            vmem((_M * _H, _D), _BF16),
            vmem((_M * _H, _D), _BF16),
            vmem((_H * _D, _M), _BF16),
            vmem((_M, _H * _D), _BF16),
            vmem((_H * _D, _M), _BF16),
            vmem((_NSLOT, _S, _D), _BF16),
            vmem((_NSLOT, _S, _D), _BF16),
            vmem((_BH, _D), _F32),
            vmem((_BH, _D), _F32),
            vmem((4 * _BH, 128), _BF16),
            vmem((_BH, _D), _F32),
            vmem((4 * _BH, 128), _F32),
            vmem((_B, _H, _M), _BF16),
            vmem((_S // _KC, _H, _KC), _F32),
            vmem((_H, _KC), _F32),
            vmem((_H, _KC), _F32),
            vmem((_B, _H, _M), _F32),
            dma((7,)), dma((_B,)), dma((_NSLOT,)), dma((_NSLOT,)), dma((len(_WO_HEADS),)),
        ],
        compiler_params=pltpu.CompilerParams(vmem_limit_bytes=100 * 2**20),
    )(
        A_x.reshape(_B, _M),
        A_c_kv,
        A_w_q.reshape(_M * _H, _D),
        A_w_uk.reshape(_M * _H, _D),
        A_w_uv.reshape(_M * _H, _D),
        A_w_o.reshape(_H * _D, _M),
        B_x.reshape(_B, _M),
        B_k_cache.reshape(_BH, _S, _D),
        B_v_cache.reshape(_BH, _S, _D),
        B_wq,
        B_wo,
    )
    return out.reshape(_B, 1, 2 * _M)
```

```python
import jax
import jax.numpy as jnp
from jax import lax
from jax.experimental import pallas as pl
from jax.experimental.pallas import tpu as pltpu

_B = 2
_H = 32
_D = 128
_M = 512
_S = 4096
_BH = _B * _H

_AHEAD = 2
_NSLOT = _AHEAD + 1
_NC = 8
_PHASE = 8
_PIECE = 16384
_UNROLL = 4
_KC = 512
_WO_HEADS = (16, 8, 4, 3, 1)
_WO_START = tuple(sum(_WO_HEADS[:g]) for g in range(len(_WO_HEADS)))

_F32 = jnp.float32
_BF16 = jnp.bfloat16
_NT = (((1,), (1,)), ((), ()))


def _dot(a, b):
    return jnp.dot(a, b, preferred_element_type=_F32)


def _dot_nt(a, b):
    return lax.dot_general(a, b, _NT, preferred_element_type=_F32)


def _iota(shape, dim):
    return lax.broadcasted_iota(jnp.int32, shape, dim)


def _ds(index, size):
    start = index * size
    return pl.ds(start if isinstance(start, int) else pl.multiple_of(start, size), size)


def _piece(ref, n):
    rows, cols = ref.shape
    if cols * 16 <= _PIECE:
        return ref.at[_ds(n, _PIECE // cols)]
    per_row = cols * 16 // _PIECE
    return ref.at[_ds(n // per_row, 16), _ds(n % per_row, _PIECE // 16)]


def _start(src, dst, sem, n, priority):
    pltpu.make_async_copy(_piece(src, n), _piece(dst, n), sem).start(priority=priority)


def _start_part(src, dst, sem, first, count):
    def pair(j, _):
        for priority in range(2):
            _start(src, dst, sem, 2 * (first + j) + priority, priority)
    lax.fori_loop(0, count, pair, None, unroll=min(_UNROLL, count))


def _wait_filled(dst, sem):
    pltpu.make_async_copy(dst, dst, sem).wait()


def _same_head_mask():
    shape = (4 * _BH, 128)
    return (_iota(shape, 0) & (_H - 1)) == (_iota(shape, 1) & (_H - 1))


def _w_rows(w_ref, a, j):
    return w_ref[_ds(a * _H + j, 128), :]


def _stack_columns(x):
    return jnp.concatenate([x[:, a * 128:(a + 1) * 128] for a in range(4)], axis=0)


def _contract_step(j, acc, lhs, w_ref):
    src_minus_cl = _iota((128, 128), 0) - (_iota((128, 128), 1) >> 5)
    spread = jnp.where(src_minus_cl == 4 * j, 1.0, 0.0).astype(_BF16)
    e = jnp.where(_same_head_mask(), _dot(lhs, spread), 0.0).astype(_BF16)
    for a in range(4):
        acc = acc + _dot(e[a * _BH:(a + 1) * _BH], _w_rows(w_ref, a, j))
    return acc


def _project_step(j, acc, q, w_ref):
    t = jnp.concatenate([_dot_nt(q, _w_rows(w_ref, a, j)) for a in range(4)], axis=0)
    t = jnp.where(_same_head_mask(), t, 0.0).astype(_BF16)
    dst_minus_cl = _iota((128, 128), 1) - (_iota((128, 128), 0) >> 5)
    gather = jnp.where(dst_minus_cl == 4 * j, 1.0, 0.0).astype(_BF16)
    return acc + _dot(t, gather)


def _out_proj(ctx_ref, w_ref, h0, nh):
    heads = [ctx_ref[pl.ds(h, _B, stride=_H), :] for h in range(h0, h0 + nh)]
    flat = jnp.concatenate(heads, axis=1).astype(_BF16)
    return _dot(flat, w_ref[pl.ds(h0 * _D, nh * _D), :])


def _kernel(ax_hbm, ckv_hbm, awq_hbm, awuk_hbm, awuv_hbm, awo_hbm,
            bx_hbm, k_hbm, v_hbm, bwq_hbm, bwo_hbm,
            out_ref,
            ax_v, bx_v, ckv_v, awq_v, awuk_v, awuv_v, awo_v, bwq_v, bwo_v, kv_v,
            qb_s, ob_s, lhs_s, acc_s, qa_acc_s, qa_s, s_s, m_s, l_s, lat_s,
            sem_in, sem_ckv, sem_k, sem_v, sem_bwo):
    scale = _D ** -0.5
    cp_ax = pltpu.make_async_copy(ax_hbm, ax_v, sem_in.at[0])
    cp_bx = pltpu.make_async_copy(bx_hbm, bx_v, sem_in.at[1])
    sem_bwq, sem_awq, sem_awuk, sem_awuv, sem_awo = (sem_in.at[n] for n in range(2, 7))
    weight_pairs = _M * _H * _D // _PIECE // 2

    kv_pairs = _S * _D // _PIECE

    def start_kv(i, n):
        slot = i % _NSLOT
        _start(k_hbm.at[i], kv_v.at[slot, 0], sem_k.at[slot], n, 0)
        _start(v_hbm.at[i], kv_v.at[slot, 1], sem_v.at[slot], n, 1)

    def start_heads(first, last):
        lax.fori_loop(first * kv_pairs, last * kv_pairs,
                      lambda j, _: start_kv(j // kv_pairs, j % kv_pairs), None, unroll=_UNROLL)

    cp_bx.start()
    cp_ax.start()
    _start_part(bwq_hbm, bwq_v, sem_bwq, 0, weight_pairs)
    start_heads(0, 2)

    cp_bx.wait()
    _wait_filled(bwq_v, sem_bwq)
    qb = _dot(bx_v[...], bwq_v[...])
    for h in range(_H):
        qb_s[pl.ds(h, _B, stride=_H), :] = qb[:, h * _D:(h + 1) * _D]
    start_heads(2, _AHEAD)

    def fetch(src, dst, sem, t):
        _start_part(src, dst, sem, t * (weight_pairs // _PHASE), weight_pairs // _PHASE)

    def contract(w_ref, t):
        n = _H // _PHASE
        lhs = lhs_s[...]
        acc_s[...] = lax.fori_loop(
            t * n, (t + 1) * n, lambda j, acc: _contract_step(j, acc, lhs, w_ref), acc_s[...])

    def a_query(t):
        @pl.when(t == 0)
        def _():
            cp_ax.wait()
            _wait_filled(awq_v, sem_awq)
            x = ax_v[...].astype(_F32)
            x_rows = jnp.concatenate(
                [jnp.broadcast_to(x[b:b + 1], (_H, _M)) for b in range(_B)], axis=0)
            lhs_s[...] = _stack_columns(x_rows).astype(_BF16)
            acc_s[...] = jnp.zeros(acc_s.shape, _F32)

        contract(awq_v, t)

    def a_absorb(t):
        @pl.when(t == 0)
        def _():
            _wait_filled(awuk_v, sem_awuk)
            qa_acc_s[...] = jnp.zeros(qa_acc_s.shape, _F32)

        n = _H // _PHASE
        q = acc_s[...].astype(_BF16)
        qa_acc_s[...] = lax.fori_loop(
            t * n, (t + 1) * n, lambda j, acc: _project_step(j, acc, q, awuk_v), qa_acc_s[...])

        @pl.when(t == _PHASE - 1)
        def _():
            for b in range(_B):
                qa_s[b] = jnp.concatenate(
                    [qa_acc_s[pl.ds(a * _BH + b * _H, _H), :] for a in range(4)],
                    axis=1).astype(_BF16)

    def a_attend(b, t):
        half = _PHASE // 2
        n = _S // _KC // half

        @pl.when(t == 0)
        def _():
            _wait_filled(ckv_v.at[b], sem_ckv.at[b])
            m_s[...] = jnp.full(m_s.shape, -jnp.inf, _F32)

        @pl.when(t < half)
        def _():
            qa = qa_s[b]

            def scores(c, m):
                s = _dot_nt(qa, ckv_v[b, _ds(c, _KC), :]) * scale
                s_s[c] = s
                return jnp.maximum(m, s)

            m_s[...] = lax.fori_loop(t * n, (t + 1) * n, scores, m_s[...])

        @pl.when(t == half)
        def _():
            m_s[...] = jnp.broadcast_to(jnp.max(m_s[...], axis=1, keepdims=True), m_s.shape)
            l_s[...] = jnp.zeros(l_s.shape, _F32)
            lat_s[b] = jnp.zeros((_H, _M), _F32)

        @pl.when(t >= half)
        def _():
            m = m_s[...]

            def values(c, carry):
                l, acc = carry
                p = jnp.exp(s_s[c] - m)
                return l + p, acc + _dot(p.astype(_BF16), ckv_v[b, _ds(c, _KC), :])

            l_s[...], lat_s[b] = lax.fori_loop(
                (t - half) * n, (t - half + 1) * n, values, (l_s[...], lat_s[b]))

        @pl.when(t == _PHASE - 1)
        def _():
            lat_s[b] = lat_s[b] / jnp.sum(l_s[...], axis=1, keepdims=True)

    def a_values(t):
        @pl.when(t == 0)
        def _():
            _wait_filled(awuv_v, sem_awuv)
            lat = jnp.concatenate([lat_s[b] for b in range(_B)], axis=0)
            lhs_s[...] = _stack_columns(lat).astype(_BF16)
            acc_s[...] = jnp.zeros(acc_s.shape, _F32)

        contract(awuv_v, t)

    def a_output():
        _wait_filled(awo_v, sem_awo)
        out_ref[:, :_M] = _out_proj(acc_s, awo_v, 0, _H).astype(out_ref.dtype)

    def head(i, issue):
        slot = i % _NSLOT
        kc = _S // _NC
        q = jnp.broadcast_to(qb_s[pl.ds(i, 1), :], (8, _D)).astype(_BF16)
        _wait_filled(kv_v.at[slot, 0], sem_k.at[slot])
        s = []
        for c in range(_NC):
            s.append(_dot_nt(q, kv_v[slot, 0, _ds(c, kc), :]))
            issue(c)
        s = jnp.concatenate(s, axis=1) * scale
        p = jnp.exp(s - jnp.max(s, axis=1, keepdims=True))
        l = jnp.sum(p, axis=1, keepdims=True)
        p = p.astype(_BF16)
        _wait_filled(kv_v.at[slot, 1], sem_v.at[slot])
        o = jnp.zeros((8, _D), _F32)
        for c in range(_NC):
            o = o + _dot(p[:, c * kc:(c + 1) * kc], kv_v[slot, 1, _ds(c, kc), :])
            issue(_NC + c)
        ob_s[pl.ds(i, 1), :] = (o / l)[0:1]

    def step(i, carry):
        def issue(g):
            n = kv_pairs // (2 * _NC)
            for j in range(g * n, (g + 1) * n):
                start_kv(i + _AHEAD, j)

        head(i, issue)
        phase, t = i // _PHASE, i % _PHASE

        @pl.when(phase == 0)
        def _():
            fetch(awq_hbm, awq_v, sem_awq, t)

        @pl.when(phase == 1)
        def _():
            a_query(t)
            fetch(awuk_hbm, awuk_v, sem_awuk, t)

        @pl.when(phase == 2)
        def _():
            a_absorb(t)

        @pl.when(jnp.logical_or(phase == 3, phase == 4))
        def _():
            a_attend(phase - 3, t)

        @pl.when(jnp.logical_or(phase == 2, phase == 3))
        def _():
            fetch(ckv_hbm.at[phase - 2], ckv_v.at[phase - 2], sem_ckv.at[phase - 2], t)

        @pl.when(phase == 4)
        def _():
            fetch(awuv_hbm, awuv_v, sem_awuv, t)

        @pl.when(phase == 5)
        def _():
            a_values(t)
            fetch(awo_hbm, awo_v, sem_awo, t)

        pl.when(i == 6 * _PHASE)(a_output)
        return carry

    lax.fori_loop(0, _BH - _AHEAD, step, 0)

    per_head = _D * _M // _PIECE

    def last_step(r, carry):
        def issue(g):
            n = _H * per_head // _AHEAD // (2 * _NC)
            for j in range(n):
                piece = (r * 2 * _NC + g) * n + j
                chunk = sum((piece >= h0 * per_head).astype(jnp.int32) for h0 in _WO_START[1:])
                _start(bwo_hbm, bwo_v, sem_bwo.at[chunk], piece, j % 2)

        head(_BH - _AHEAD + r, issue)
        return carry

    lax.fori_loop(0, _AHEAD, last_step, 0)

    acc = jnp.zeros((_B, _M), _F32)
    for g in range(len(_WO_HEADS)):
        _wait_filled(bwo_v.at[pl.ds(_WO_START[g] * _D, _WO_HEADS[g] * _D)], sem_bwo.at[g])
        acc = acc + _out_proj(ob_s, bwo_v, _WO_START[g], _WO_HEADS[g])
    out_ref[:, _M:] = acc.astype(out_ref.dtype)


@jax.jit
def pallas_concat_heads__compressed_kv_cla__gqa_block_cached__decode_kernel(
    A_x: jax.Array,
    A_c_kv: jax.Array,
    A_w_q: jax.Array,
    A_w_uk: jax.Array,
    A_w_uv: jax.Array,
    A_w_o: jax.Array,
    B_x: jax.Array,
    B_k_cache: jax.Array,
    B_v_cache: jax.Array,
    B_wq: jax.Array,
    B_wo: jax.Array,
):
    assert A_x.shape == (_B, 1, _M) and B_x.shape == (_B, 1, _M)
    assert A_c_kv.shape == (_B, _S, _M)
    assert A_w_q.shape == A_w_uk.shape == A_w_uv.shape == (_M, _H, _D)
    assert A_w_o.shape == (_H, _D, _M)
    assert B_k_cache.shape == B_v_cache.shape == (_B, _H, _S, _D)
    assert B_wq.shape == (_M, _H * _D) and B_wo.shape == (_H * _D, _M)

    vmem = pltpu.VMEM
    dma = pltpu.SemaphoreType.DMA
    out = pl.pallas_call(
        _kernel,
        in_specs=[pl.BlockSpec(memory_space=pltpu.HBM)] * 11,
        out_specs=pl.BlockSpec(memory_space=vmem),
        out_shape=jax.ShapeDtypeStruct((_B, 2 * _M), A_x.dtype),
        scratch_shapes=[
            vmem((_B, _M), _BF16),
            vmem((_B, _M), _BF16),
            vmem((_B, _S, _M), _BF16),
            vmem((_M * _H, _D), _BF16),
            vmem((_M * _H, _D), _BF16),
            vmem((_M * _H, _D), _BF16),
            vmem((_H * _D, _M), _BF16),
            vmem((_M, _H * _D), _BF16),
            vmem((_H * _D, _M), _BF16),
            vmem((_NSLOT, 2, _S, _D), _BF16),
            vmem((_BH, _D), _F32),
            vmem((_BH, _D), _F32),
            vmem((4 * _BH, 128), _BF16),
            vmem((_BH, _D), _F32),
            vmem((4 * _BH, 128), _F32),
            vmem((_B, _H, _M), _BF16),
            vmem((_S // _KC, _H, _KC), _F32),
            vmem((_H, _KC), _F32),
            vmem((_H, _KC), _F32),
            vmem((_B, _H, _M), _F32),
            dma((7,)), dma((_B,)), dma((_NSLOT,)), dma((_NSLOT,)), dma((len(_WO_HEADS),)),
        ],
        compiler_params=pltpu.CompilerParams(vmem_limit_bytes=100 * 2**20),
    )(
        A_x.reshape(_B, _M),
        A_c_kv,
        A_w_q.reshape(_M * _H, _D),
        A_w_uk.reshape(_M * _H, _D),
        A_w_uv.reshape(_M * _H, _D),
        A_w_o.reshape(_H * _D, _M),
        B_x.reshape(_B, _M),
        B_k_cache.reshape(_BH, _S, _D),
        B_v_cache.reshape(_BH, _S, _D),
        B_wq,
        B_wo,
    )
    return out.reshape(_B, 1, 2 * _M)
```

```python
import jax
import jax.numpy as jnp
from jax import lax
from jax.experimental import pallas as pl
from jax.experimental.pallas import tpu as pltpu

_B = 2
_H = 32
_D = 128
_M = 512
_S = 4096
_BH = _B * _H

_PIECE = 16384
_NB = 4
_G = 8
_LAG = 64
_NC = 8
_KC = 512
_STAGE_PAIRS = 4
_STAGE_UNROLL = 1
_PIN_A = False
_PIN_LAST = True
_EARLY_CHUNKS = 6

_W_PAIRS = _M * _H * _D // _PIECE
_HEAD_PAIRS = _S * _D // _PIECE
_HEADS_START = _W_PAIRS + _LAG + 4 * _H * _STAGE_PAIRS
_AHEAD = (_HEADS_START - 3 * _W_PAIRS) // _HEAD_PAIRS
_NSLOT = (_AHEAD + _G - 1) // _G + 1
assert _AHEAD * _HEAD_PAIRS >= _G * _HEAD_PAIRS + _LAG

_WQ, _WUK, _WUV, _RING = 0, _NB, 2 * _NB, 3 * _NB
_NARROW_SPARE = _RING + _NSLOT * 2 * _G
_CKV, _AWO, _BWO, _WIDE_SPARE = 0, _B * _NB, (_B + 1) * _NB, (_B + 2) * _NB

_F32 = jnp.float32
_BF16 = jnp.bfloat16
_NT = (((1,), (1,)), ((), ()))


def _dot(a, b):
    return jnp.dot(a, b, preferred_element_type=_F32)


def _dot_nt(a, b):
    return lax.dot_general(a, b, _NT, preferred_element_type=_F32)


def _iota(shape, dim):
    return lax.broadcasted_iota(jnp.int32, shape, dim)


def _ds(index, size):
    start = index * size
    return pl.ds(start if isinstance(start, int) else pl.multiple_of(start, size), size)


def _wait_filled(dst, sem):
    pltpu.make_async_copy(dst, dst, sem).wait()


def _same_head_mask():
    shape = (_NB * _BH, 128)
    return (_iota(shape, 0) & (_H - 1)) == (_iota(shape, 1) & (_H - 1))


def _stack_columns(x):
    return jnp.concatenate([x[:, a * 128:(a + 1) * 128] for a in range(_NB)], axis=0)


def _contract_step(j, acc, lhs, w_rows, issue):
    src_minus_cl = _iota((128, 128), 0) - (_iota((128, 128), 1) >> 5)
    spread = jnp.where(src_minus_cl == 4 * j, 1.0, 0.0).astype(_BF16)
    e = jnp.where(_same_head_mask(), _dot(lhs, spread), 0.0).astype(_BF16)
    for a in range(_NB):
        part = _dot(e[a * _BH:(a + 1) * _BH], w_rows(a, j))
        issue(a, _NB, part)
        acc = acc + part
    return acc


def _project_step(j, acc, q, w_rows, issue):
    t = []
    for a in range(_NB):
        t.append(_dot_nt(q, w_rows(a, j)))
        issue(a, _NB, t[-1])
    t = jnp.where(_same_head_mask(), jnp.concatenate(t, axis=0), 0.0).astype(_BF16)
    dst_minus_cl = _iota((128, 128), 1) - (_iota((128, 128), 0) >> 5)
    gather = jnp.where(dst_minus_cl == 4 * j, 1.0, 0.0).astype(_BF16)
    return acc + _dot(t, gather)


def _kernel(ax_hbm, ckv_hbm, awq_hbm, awuk_hbm, awuv_hbm, awo_hbm,
            bx_hbm, k_hbm, v_hbm, bwq_hbm, bwo_hbm,
            out_ref,
            ax_v, bx_v, bwq_v, narrow_v, wide_v, qb_s, ob_s, ctx_s, s_s,
            sem_x, sem_w, sem_k, sem_v, sem_wo):
    scale = _D ** -0.5
    sem_bwq, sem_wq, sem_wuk, sem_wuv, sem_ckv0, sem_ckv1 = (sem_w.at[n] for n in range(6))
    heads_per_block = _H // _NB

    def start_rows(src, buf, block, sem, n, priority):
        rows = _ds(n, _PIECE // _NB // src.shape[-1])
        pltpu.make_async_copy(
            src.at[:, rows], buf.at[pl.ds(block, _NB), rows], sem).start(priority=priority)

    def start_queries(n):
        cols = _PIECE // _NB // 16
        per_row = _H * _D // cols
        piece = (slice(None), _ds(n // per_row, 16), _ds(n % per_row, cols))
        pltpu.make_async_copy(bwq_hbm.at[piece], bwq_v.at[piece], sem_bwq).start(priority=0)
        start_rows(awq_hbm, narrow_v, _WQ, sem_wq, n, 1)

    def start_up_projections(n):
        start_rows(awuk_hbm, narrow_v, _WUK, sem_wuk, n, 0)
        start_rows(awuv_hbm, narrow_v, _WUV, sem_wuv, n, 1)

    def start_latents(n):
        start_rows(ckv_hbm.at[0], wide_v, _CKV, sem_ckv0, n, 0)
        start_rows(ckv_hbm.at[1], wide_v, _CKV + _NB, sem_ckv1, n, 1)

    def ring_block(group, is_v):
        return _RING + ((group % _NSLOT) * 2 + is_v) * _G

    def start_kv(n):
        group = n // (_G * _HEAD_PAIRS)
        rows = _ds(n % (_G * _HEAD_PAIRS), _PIECE // _G // _D)
        for is_v, (src, sem) in enumerate(((k_hbm, sem_k), (v_hbm, sem_v))):
            pltpu.make_async_copy(
                src.at[_ds(group, _G), rows],
                narrow_v.at[pl.ds(ring_block(group, is_v), _G), rows],
                sem.at[group % _NSLOT]).start(priority=is_v)

    def start_out_projections(n):
        t = n // (_W_PAIRS // heads_per_block)
        start_rows(awo_hbm, wide_v, _AWO, sem_wo.at[0, t], n, 0)
        start_rows(bwo_hbm, wide_v, _BWO, sem_wo.at[1, t], n, 1)

    stream = ((_W_PAIRS, start_queries, None),
              (_W_PAIRS, start_up_projections, (narrow_v, _NARROW_SPARE)),
              (_W_PAIRS, start_latents, (wide_v, _WIDE_SPARE)),
              (_BH * _HEAD_PAIRS, start_kv, (narrow_v, _NARROW_SPARE)),
              (_W_PAIRS, start_out_projections, (wide_v, _WIDE_SPARE)))
    started = [0]

    def streaming_loop(lo, hi, pairs, body, carry, unroll=1, pin=False):
        while lo < hi:
            first = started[0]
            for length, start, spare in stream:
                if first < length:
                    break
                first -= length
            steps = min(hi - lo, (length - first) // pairs)
            assert steps > 0

            def step(j, carry, lo=lo, first=first, start=start, spare=spare):
                def issue(g, n, after=None):
                    todo = range(g * pairs // n, (g + 1) * pairs // n)
                    if pin and todo:
                        spare[0][spare[1], :16, :128] = after[:16, :128].astype(_BF16)
                    for k in todo:
                        start(first + (j - lo) * pairs + k)
                return body(j, carry, issue)

            carry = lax.fori_loop(lo, lo + steps, step, carry, unroll=unroll)
            started[0] += steps * pairs
            lo += steps
        return carry

    def start_pairs(count):
        streaming_loop(0, count, 1, lambda j, carry, issue: issue(0, 1), None, unroll=4)

    def weight(buf, block):
        return buf.at[pl.ds(block, _NB)]

    def narrow_rows(block):
        return lambda a, j: narrow_v[block + a, _ds(j, 128), :]

    cp_ax = pltpu.make_async_copy(ax_hbm, ax_v, sem_x.at[0])
    cp_bx = pltpu.make_async_copy(bx_hbm, bx_v, sem_x.at[1])
    cp_ax.start()
    cp_bx.start()
    start_pairs(_W_PAIRS + _LAG // 2)

    cp_bx.wait()
    _wait_filled(bwq_v, sem_bwq)
    qb = _dot(bx_v[...], bwq_v[...].reshape(_M, _H * _D))
    for h in range(_H):
        qb_s[pl.ds(h, _B, stride=_H), :] = qb[:, h * _D:(h + 1) * _D]
    start_pairs(_LAG // 2)

    def per_head_contract(lhs, block):
        lhs = _stack_columns(lhs).astype(_BF16)
        return streaming_loop(
            0, _H, _STAGE_PAIRS,
            lambda j, acc, issue: _contract_step(j, acc, lhs, narrow_rows(block), issue),
            jnp.zeros((_BH, _D), _F32), _STAGE_UNROLL, _PIN_A)

    cp_ax.wait()
    _wait_filled(weight(narrow_v, _WQ), sem_wq)
    x = ax_v[...].astype(_F32)
    x_rows = jnp.concatenate(
        [jnp.broadcast_to(x[b:b + 1], (_H, _M)) for b in range(_B)], axis=0)
    q = per_head_contract(x_rows, _WQ).astype(_BF16)

    _wait_filled(weight(narrow_v, _WUK), sem_wuk)
    qa = streaming_loop(
        0, _H, _STAGE_PAIRS,
        lambda j, acc, issue: _project_step(j, acc, q, narrow_rows(_WUK), issue),
        jnp.zeros((_NB * _BH, 128), _F32), _STAGE_UNROLL, _PIN_A)

    latents = []
    for b, sem in enumerate((sem_ckv0, sem_ckv1)):
        qa_b = jnp.concatenate(
            [qa[a * _BH + b * _H:a * _BH + (b + 1) * _H] for a in range(_NB)],
            axis=1).astype(_BF16)
        steps_per_block = _S // _NB // _KC
        parts = _KC // 128

        def keys(c, part, b=b):
            return wide_v[_CKV + b * _NB + c // steps_per_block,
                          _ds((c % steps_per_block) * parts + part, 128), :]

        def scores(c, m, issue, qa_b=qa_b, keys=keys):
            s = []
            for part in range(parts):
                s.append(_dot_nt(qa_b, keys(c, part)))
                issue(part, parts, s[-1])
            s = jnp.concatenate(s, axis=1) * scale
            s_s[c] = s
            return jnp.maximum(m, s)

        _wait_filled(weight(wide_v, _CKV + b * _NB), sem)
        m = streaming_loop(0, _S // _KC, _STAGE_PAIRS, scores,
                           jnp.full((_H, _KC), -jnp.inf, _F32), 1, _PIN_A)
        m = jnp.max(m, axis=1, keepdims=True)

        def values(c, carry, issue, m=m, keys=keys):
            l, acc = carry
            p = jnp.exp(s_s[c] - m)
            l = l + p
            p = p.astype(_BF16)
            for part in range(parts):
                o = _dot(p[:, part * 128:(part + 1) * 128], keys(c, part))
                issue(part, parts, o)
                acc = acc + o
            return l, acc

        l, acc = streaming_loop(0, _S // _KC, _STAGE_PAIRS, values,
                                (jnp.zeros((_H, _KC), _F32), jnp.zeros((_H, _M), _F32)), 1, _PIN_A)
        latents.append(acc / jnp.sum(l, axis=1, keepdims=True))

    _wait_filled(weight(narrow_v, _WUV), sem_wuv)
    ctx_s[...] = per_head_contract(jnp.concatenate(latents, axis=0), _WUV)

    def head(i, carry, issue):
        group, member = i // _G, i % _G
        k_block, v_block = ring_block(group, 0), ring_block(group, 1)
        kc = _S // _NC

        @pl.when(member == 0)
        def _():
            _wait_filled(narrow_v.at[pl.ds(k_block, _G)], sem_k.at[group % _NSLOT])
            _wait_filled(narrow_v.at[pl.ds(v_block, _G)], sem_v.at[group % _NSLOT])

        q = jnp.broadcast_to(qb_s[pl.ds(i, 1), :], (16, _D)).astype(_BF16)
        s = []
        for c in range(_NC):
            s.append(_dot_nt(q, narrow_v[k_block + member, _ds(c, kc), :]))
            issue(c, 2 * _NC, s[-1])
        s = jnp.concatenate([part[:8] for part in s], axis=1) * scale
        p = jnp.exp(s - jnp.max(s, axis=1, keepdims=True))
        l = jnp.sum(p, axis=1, keepdims=True)
        p = jnp.concatenate([p, p], axis=0).astype(_BF16)
        o = jnp.zeros((16, _D), _F32)
        for c in range(_NC):
            part = _dot(p[:, c * kc:(c + 1) * kc], narrow_v[v_block + member, _ds(c, kc), :])
            issue(_NC + c, 2 * _NC, part)
            o = o + part
        ob_s[pl.ds(i, 1), :] = (o[:8] / l)[0:1]
        return carry

    assert started[0] == _HEADS_START
    streaming_loop(0, _BH - _AHEAD, _HEAD_PAIRS, head, None)
    few, extra = divmod(_W_PAIRS, _AHEAD)
    for lo, hi, pairs in ((_BH - _AHEAD, _BH - _AHEAD + extra, few + 1),
                          (_BH - _AHEAD + extra, _BH, few)):
        streaming_loop(lo, hi, pairs, head, None, 1, _PIN_LAST)
    assert started[0] == sum(length for length, _, _ in stream)

    def out_proj(ctx_ref, block, t):
        acc = jnp.zeros((_B, _M), _F32)
        for a in range(_NB):
            ctx = ctx_ref[pl.ds(a * heads_per_block + t, _B, stride=_H), :]
            acc = acc + _dot(ctx.astype(_BF16), wide_v[block + a, _ds(t, _D), :])
        return acc

    early, late = range(_EARLY_CHUNKS), range(_EARLY_CHUNKS, heads_per_block)
    out = [jnp.zeros((_B, _M), _F32)] * 2
    for branch, chunks in ((0, early), (1, early), (0, late), (1, late)):
        ctx_ref, block = ((ctx_s, _AWO), (ob_s, _BWO))[branch]
        for t in chunks:
            _wait_filled(wide_v.at[pl.ds(block, _NB), _ds(t, _D)], sem_wo.at[branch, t])
            out[branch] = out[branch] + out_proj(ctx_ref, block, t)
    out_ref[...] = jnp.concatenate(out, axis=1).astype(out_ref.dtype)


@jax.jit
def pallas_concat_heads__compressed_kv_cla__gqa_block_cached__decode_kernel(
    A_x: jax.Array,
    A_c_kv: jax.Array,
    A_w_q: jax.Array,
    A_w_uk: jax.Array,
    A_w_uv: jax.Array,
    A_w_o: jax.Array,
    B_x: jax.Array,
    B_k_cache: jax.Array,
    B_v_cache: jax.Array,
    B_wq: jax.Array,
    B_wo: jax.Array,
):
    assert A_x.shape == (_B, 1, _M) and B_x.shape == (_B, 1, _M)
    assert A_c_kv.shape == (_B, _S, _M)
    assert A_w_q.shape == A_w_uk.shape == A_w_uv.shape == (_M, _H, _D)
    assert A_w_o.shape == (_H, _D, _M)
    assert B_k_cache.shape == B_v_cache.shape == (_B, _H, _S, _D)
    assert B_wq.shape == (_M, _H * _D) and B_wo.shape == (_H * _D, _M)

    narrow = (_NB, _M * _H // _NB, _D)
    wide = (_NB, _H * _D // _NB, _M)
    vmem = pltpu.VMEM
    dma = pltpu.SemaphoreType.DMA
    out = pl.pallas_call(
        _kernel,
        in_specs=[pl.BlockSpec(memory_space=pltpu.HBM)] * 11,
        out_specs=pl.BlockSpec(memory_space=vmem),
        out_shape=jax.ShapeDtypeStruct((_B, 2 * _M), A_x.dtype),
        scratch_shapes=[
            vmem((_B, _M), _BF16),
            vmem((_B, _M), _BF16),
            vmem((_NB, _M // _NB, _H * _D), _BF16),
            vmem((_NARROW_SPARE + 1,) + narrow[1:], _BF16),
            vmem((_WIDE_SPARE + 1,) + wide[1:], _BF16),
            vmem((_BH, _D), _F32),
            vmem((_BH, _D), _F32),
            vmem((_BH, _D), _F32),
            vmem((_S // _KC, _H, _KC), _F32),
            dma((2,)), dma((6,)), dma((_NSLOT,)), dma((_NSLOT,)), dma((2, _H // _NB)),
        ],
        compiler_params=pltpu.CompilerParams(vmem_limit_bytes=110 * 2**20),
    )(
        A_x.reshape(_B, _M),
        A_c_kv.reshape((_B,) + wide),
        A_w_q.reshape(narrow),
        A_w_uk.reshape(narrow),
        A_w_uv.reshape(narrow),
        A_w_o.reshape(wide),
        B_x.reshape(_B, _M),
        B_k_cache.reshape(_BH, _S, _D),
        B_v_cache.reshape(_BH, _S, _D),
        B_wq.reshape(_NB, _M // _NB, _H * _D),
        B_wo.reshape(wide),
    )
    return out.reshape(_B, 1, 2 * _M)
```

```python
import jax
import jax.numpy as jnp
from jax import lax
from jax.experimental import pallas as pl
from jax.experimental.pallas import tpu as pltpu

_B = 2
_H = 32
_D = 128
_M = 512
_S = 4096
_BH = _B * _H

_PIECE = 16384
_NB = 4
_G = 8
_LAG = 64
_NC = 8
_KC = 512
_STAGE_PAIRS = 4
_STAGE_UNROLL = 1
_PIN_A = False
_PIN_LAST = True
_EARLY = 5
_AFTER_QUERIES = 16

_W_PAIRS = _M * _H * _D // _PIECE
_HEAD_PAIRS = _S * _D // _PIECE
_HEADS_START = _W_PAIRS + _LAG + 4 * _H * _STAGE_PAIRS
_AHEAD = (_HEADS_START - 3 * _W_PAIRS) // _HEAD_PAIRS
_NSLOT = (_AHEAD + _G - 1) // _G + 1
assert _AHEAD * _HEAD_PAIRS >= _G * _HEAD_PAIRS + _LAG

_WQ, _WUK, _WUV, _RING = 0, _NB, 2 * _NB, 3 * _NB
_NARROW_SPARE = _RING + _NSLOT * 2 * _G
_CKV, _AWO, _BWO, _WIDE_SPARE = 0, _B * _NB, (_B + 1) * _NB, (_B + 2) * _NB

_F32 = jnp.float32
_BF16 = jnp.bfloat16
_NT = (((1,), (1,)), ((), ()))


def _dot(a, b):
    return jnp.dot(a, b, preferred_element_type=_F32)


def _dot_nt(a, b):
    return lax.dot_general(a, b, _NT, preferred_element_type=_F32)


def _iota(shape, dim):
    return lax.broadcasted_iota(jnp.int32, shape, dim)


def _ds(index, size):
    start = index * size
    return pl.ds(start if isinstance(start, int) else pl.multiple_of(start, size), size)


def _wait_filled(dst, sem):
    pltpu.make_async_copy(dst, dst, sem).wait()


def _same_head_mask():
    shape = (_NB * _BH, 128)
    return (_iota(shape, 0) & (_H - 1)) == (_iota(shape, 1) & (_H - 1))


def _stack_columns(x):
    return jnp.concatenate([x[:, a * 128:(a + 1) * 128] for a in range(_NB)], axis=0)


def _contract_step(j, acc, lhs, w_rows, issue):
    src_minus_cl = _iota((128, 128), 0) - (_iota((128, 128), 1) >> 5)
    spread = jnp.where(src_minus_cl == 4 * j, 1.0, 0.0).astype(_BF16)
    e = jnp.where(_same_head_mask(), _dot(lhs, spread), 0.0).astype(_BF16)
    for a in range(_NB):
        part = _dot(e[a * _BH:(a + 1) * _BH], w_rows(a, j))
        issue(a, _NB, part)
        acc = acc + part
    return acc


def _project_step(j, acc, q, w_rows, issue):
    t = []
    for a in range(_NB):
        t.append(_dot_nt(q, w_rows(a, j)))
        issue(a, _NB, t[-1])
    t = jnp.where(_same_head_mask(), jnp.concatenate(t, axis=0), 0.0).astype(_BF16)
    dst_minus_cl = _iota((128, 128), 1) - (_iota((128, 128), 0) >> 5)
    gather = jnp.where(dst_minus_cl == 4 * j, 1.0, 0.0).astype(_BF16)
    return acc + _dot(t, gather)


def _kernel(ax_hbm, ckv_hbm, awq_hbm, awuk_hbm, awuv_hbm, awo_hbm,
            bx_hbm, k_hbm, v_hbm, bwq_hbm, bwo_hbm,
            out_ref,
            ax_v, bx_v, bwq_v, narrow_v, wide_v, qb_s, ob_s, ctx_s, s_s,
            sems):
    scale = _D ** -0.5
    heads_per_block = _H // _NB

    def start_rows(src, buf, block, sem, n, priority):
        rows = _ds(n, _PIECE // _NB // src.shape[-1])
        pltpu.make_async_copy(
            src.at[:, rows], buf.at[pl.ds(block, _NB), rows], sem).start(priority=priority)

    def start_queries(n):
        cols = _PIECE // _NB // 16
        per_row = _H * _D // cols
        piece = (slice(None), _ds(n // per_row, 16), _ds(n % per_row, cols))
        pltpu.make_async_copy(bwq_hbm.at[piece], bwq_v.at[piece], sems.at[0]).start(priority=0)
        start_rows(awq_hbm, narrow_v, _WQ, sems.at[0], n, 1)

    def start_up_projections(n):
        start_rows(awuk_hbm, narrow_v, _WUK, sems.at[1], n, 0)
        start_rows(awuv_hbm, narrow_v, _WUV, sems.at[1], n, 1)

    def start_latents(n):
        start_rows(ckv_hbm.at[0], wide_v, _CKV, sems.at[0], n, 0)
        start_rows(ckv_hbm.at[1], wide_v, _CKV + _NB, sems.at[0], n, 1)

    def ring_block(group, is_v):
        return _RING + ((group % _NSLOT) * 2 + is_v) * _G

    def start_kv(n):
        group = n // (_G * _HEAD_PAIRS)
        rows = _ds(n % (_G * _HEAD_PAIRS), _PIECE // _G // _D)
        for is_v, src in enumerate((k_hbm, v_hbm)):
            pltpu.make_async_copy(
                src.at[_ds(group, _G), rows],
                narrow_v.at[pl.ds(ring_block(group, is_v), _G), rows],
                sems.at[(group + 1) % 2]).start(priority=is_v)

    def start_out_projections(n):
        t = n // (_W_PAIRS // heads_per_block)
        start_rows(awo_hbm, wide_v, _AWO, sems.at[jnp.where(t < _EARLY, 2, 3)], n, 0)
        start_rows(bwo_hbm, wide_v, _BWO, sems.at[jnp.where(t < _EARLY, 2, t - _EARLY + 4)], n, 1)

    stream = ((_W_PAIRS, start_queries, None),
              (_W_PAIRS, start_up_projections, (narrow_v, _NARROW_SPARE)),
              (_W_PAIRS, start_latents, (wide_v, _WIDE_SPARE)),
              (_BH * _HEAD_PAIRS, start_kv, (narrow_v, _NARROW_SPARE)),
              (_W_PAIRS, start_out_projections, (wide_v, _WIDE_SPARE)))
    started = [0]

    def streaming_loop(lo, hi, pairs, body, carry, unroll=1, pin=False):
        while lo < hi:
            first = started[0]
            for length, start, spare in stream:
                if first < length:
                    break
                first -= length
            steps = min(hi - lo, (length - first) // pairs)
            assert steps > 0

            def step(j, carry, lo=lo, first=first, start=start, spare=spare):
                def issue(g, n, after=None):
                    todo = range(g * pairs // n, (g + 1) * pairs // n)
                    if pin and todo:
                        spare[0][spare[1], :16, :128] = after[:16, :128].astype(_BF16)
                    for k in todo:
                        start(first + (j - lo) * pairs + k)
                return body(j, carry, issue)

            carry = lax.fori_loop(lo, lo + steps, step, carry, unroll=unroll)
            started[0] += steps * pairs
            lo += steps
        return carry

    def start_pairs(count):
        streaming_loop(0, count, 1, lambda j, carry, issue: issue(0, 1), None, unroll=4)

    def narrow_rows(block):
        return lambda a, j: narrow_v[block + a, _ds(j, 128), :]

    cp_ax = pltpu.make_async_copy(ax_hbm, ax_v, sems.at[0])
    cp_bx = pltpu.make_async_copy(bx_hbm, bx_v, sems.at[0])
    cp_ax.start()
    cp_bx.start()
    start_pairs(_W_PAIRS + _LAG - _AFTER_QUERIES)

    cp_ax.wait()
    cp_bx.wait()
    _wait_filled(bwq_v, sems.at[0])
    _wait_filled(narrow_v.at[pl.ds(_WQ, _NB)], sems.at[0])
    qb = _dot(bx_v[...], bwq_v[...].reshape(_M, _H * _D))
    for h in range(_H):
        qb_s[pl.ds(h, _B, stride=_H), :] = qb[:, h * _D:(h + 1) * _D]
    start_pairs(_AFTER_QUERIES)

    def per_head_contract(lhs, block):
        lhs = _stack_columns(lhs).astype(_BF16)
        return streaming_loop(
            0, _H, _STAGE_PAIRS,
            lambda j, acc, issue: _contract_step(j, acc, lhs, narrow_rows(block), issue),
            jnp.zeros((_BH, _D), _F32), _STAGE_UNROLL, _PIN_A)

    x = ax_v[...].astype(_F32)
    x_rows = jnp.concatenate(
        [jnp.broadcast_to(x[b:b + 1], (_H, _M)) for b in range(_B)], axis=0)
    q = per_head_contract(x_rows, _WQ).astype(_BF16)

    _wait_filled(narrow_v.at[pl.ds(_WUK, 2 * _NB)], sems.at[1])
    qa = streaming_loop(
        0, _H, _STAGE_PAIRS,
        lambda j, acc, issue: _project_step(j, acc, q, narrow_rows(_WUK), issue),
        jnp.zeros((_NB * _BH, 128), _F32), _STAGE_UNROLL, _PIN_A)

    _wait_filled(wide_v.at[pl.ds(_CKV, _B * _NB)], sems.at[0])
    latents = []
    for b in range(_B):
        qa_b = jnp.concatenate(
            [qa[a * _BH + b * _H:a * _BH + (b + 1) * _H] for a in range(_NB)],
            axis=1).astype(_BF16)
        steps_per_block = _S // _NB // _KC
        parts = _KC // 128

        def keys(c, part, b=b):
            return wide_v[_CKV + b * _NB + c // steps_per_block,
                          _ds((c % steps_per_block) * parts + part, 128), :]

        def scores(c, m, issue, qa_b=qa_b, keys=keys):
            s = []
            for part in range(parts):
                s.append(_dot_nt(qa_b, keys(c, part)))
                issue(part, parts, s[-1])
            s = jnp.concatenate(s, axis=1) * scale
            s_s[c] = s
            return jnp.maximum(m, s)

        m = streaming_loop(0, _S // _KC, _STAGE_PAIRS, scores,
                           jnp.full((_H, _KC), -jnp.inf, _F32), 1, _PIN_A)
        m = jnp.max(m, axis=1, keepdims=True)

        def values(c, carry, issue, m=m, keys=keys):
            l, acc = carry
            p = jnp.exp(s_s[c] - m)
            l = l + p
            p = p.astype(_BF16)
            for part in range(parts):
                o = _dot(p[:, part * 128:(part + 1) * 128], keys(c, part))
                issue(part, parts, o)
                acc = acc + o
            return l, acc

        l, acc = streaming_loop(0, _S // _KC, _STAGE_PAIRS, values,
                                (jnp.zeros((_H, _KC), _F32), jnp.zeros((_H, _M), _F32)), 1, _PIN_A)
        latents.append(acc / jnp.sum(l, axis=1, keepdims=True))

    ctx_s[...] = per_head_contract(jnp.concatenate(latents, axis=0), _WUV)

    def head(i, carry, issue):
        group, member = i // _G, i % _G
        k_block, v_block = ring_block(group, 0), ring_block(group, 1)
        kc = _S // _NC

        @pl.when(member == 0)
        def _():
            _wait_filled(narrow_v.at[pl.ds(k_block, 2 * _G)], sems.at[(group + 1) % 2])

        q = jnp.broadcast_to(qb_s[pl.ds(i, 1), :], (16, _D)).astype(_BF16)
        s = []
        for c in range(_NC):
            s.append(_dot_nt(q, narrow_v[k_block + member, _ds(c, kc), :]))
            issue(c, 2 * _NC, s[-1])
        s = jnp.concatenate([part[:8] for part in s], axis=1) * scale
        p = jnp.exp(s - jnp.max(s, axis=1, keepdims=True))
        l = jnp.sum(p, axis=1, keepdims=True)
        p = jnp.concatenate([p, p], axis=0).astype(_BF16)
        o = jnp.zeros((16, _D), _F32)
        for c in range(_NC):
            part = _dot(p[:, c * kc:(c + 1) * kc], narrow_v[v_block + member, _ds(c, kc), :])
            issue(_NC + c, 2 * _NC, part)
            o = o + part
        ob_s[pl.ds(i, 1), :] = (o[:8] / l)[0:1]
        return carry

    assert started[0] == _HEADS_START
    streaming_loop(0, _BH - _AHEAD, _HEAD_PAIRS, head, None)
    few, extra = divmod(_W_PAIRS, _AHEAD)
    for lo, hi, pairs in ((_BH - _AHEAD, _BH - _AHEAD + extra, few + 1),
                          (_BH - _AHEAD + extra, _BH, few)):
        streaming_loop(lo, hi, pairs, head, None, 1, _PIN_LAST)
    assert started[0] == sum(length for length, _, _ in stream)

    def out_proj(ctx_ref, block, t):
        acc = jnp.zeros((_B, _M), _F32)
        for a in range(_NB):
            ctx = ctx_ref[pl.ds(a * heads_per_block + t, _B, stride=_H), :]
            acc = acc + _dot(ctx.astype(_BF16), wide_v[block + a, _ds(t, _D), :])
        return acc

    def wait_heads(block, first, count, sem):
        _wait_filled(wide_v.at[pl.ds(block, _NB), pl.ds(first * _D, count * _D)], sems.at[sem])

    wait_heads(_AWO, 0, _EARLY, 2)
    wait_heads(_BWO, 0, _EARLY, 2)
    out_a = sum(out_proj(ctx_s, _AWO, t) for t in range(_EARLY))
    out_b = sum(out_proj(ob_s, _BWO, t) for t in range(_EARLY))
    wait_heads(_AWO, _EARLY, heads_per_block - _EARLY, 3)
    out_a = out_a + sum(out_proj(ctx_s, _AWO, t) for t in range(_EARLY, heads_per_block))
    out_ref[:, :_M] = out_a.astype(out_ref.dtype)
    for t in range(_EARLY, heads_per_block):
        wait_heads(_BWO, t, 1, t - _EARLY + 4)
        out_b = out_b + out_proj(ob_s, _BWO, t)
    out_ref[:, _M:] = out_b.astype(out_ref.dtype)


@jax.jit
def pallas_concat_heads__compressed_kv_cla__gqa_block_cached__decode_kernel(
    A_x: jax.Array,
    A_c_kv: jax.Array,
    A_w_q: jax.Array,
    A_w_uk: jax.Array,
    A_w_uv: jax.Array,
    A_w_o: jax.Array,
    B_x: jax.Array,
    B_k_cache: jax.Array,
    B_v_cache: jax.Array,
    B_wq: jax.Array,
    B_wo: jax.Array,
):
    assert A_x.shape == (_B, 1, _M) and B_x.shape == (_B, 1, _M)
    assert A_c_kv.shape == (_B, _S, _M)
    assert A_w_q.shape == A_w_uk.shape == A_w_uv.shape == (_M, _H, _D)
    assert A_w_o.shape == (_H, _D, _M)
    assert B_k_cache.shape == B_v_cache.shape == (_B, _H, _S, _D)
    assert B_wq.shape == (_M, _H * _D) and B_wo.shape == (_H * _D, _M)

    narrow = (_NB, _M * _H // _NB, _D)
    wide = (_NB, _H * _D // _NB, _M)
    vmem = pltpu.VMEM
    dma = pltpu.SemaphoreType.DMA
    out = pl.pallas_call(
        _kernel,
        in_specs=[pl.BlockSpec(memory_space=pltpu.HBM)] * 11,
        out_specs=pl.BlockSpec(memory_space=vmem),
        out_shape=jax.ShapeDtypeStruct((_B, 2 * _M), A_x.dtype),
        scratch_shapes=[
            vmem((_B, _M), _BF16),
            vmem((_B, _M), _BF16),
            vmem((_NB, _M // _NB, _H * _D), _BF16),
            vmem((_NARROW_SPARE + 1,) + narrow[1:], _BF16),
            vmem((_WIDE_SPARE + 1,) + wide[1:], _BF16),
            vmem((_BH, _D), _F32),
            vmem((_BH, _D), _F32),
            vmem((_BH, _D), _F32),
            vmem((_S // _KC, _H, _KC), _F32),
            dma((4 + _H // _NB - _EARLY,)),
        ],
        compiler_params=pltpu.CompilerParams(vmem_limit_bytes=110 * 2**20),
    )(
        A_x.reshape(_B, _M),
        A_c_kv.reshape((_B,) + wide),
        A_w_q.reshape(narrow),
        A_w_uk.reshape(narrow),
        A_w_uv.reshape(narrow),
        A_w_o.reshape(wide),
        B_x.reshape(_B, _M),
        B_k_cache.reshape(_BH, _S, _D),
        B_v_cache.reshape(_BH, _S, _D),
        B_wq.reshape(_NB, _M // _NB, _H * _D),
        B_wo.reshape(wide),
    )
    return out.reshape(_B, 1, 2 * _M)
```

```python
import jax
import jax.numpy as jnp
from jax import lax
from jax.experimental import pallas as pl
from jax.experimental.pallas import tpu as pltpu

_B = 2
_H = 32
_D = 128
_M = 512
_S = 4096
_BH = _B * _H

_PIECE = 16384
_NB = 4
_G = 8
_LAG = 64
_NC = 8
_KC = 512
_STAGE_PAIRS = 4
_EARLY = 5

_W_PAIRS = _M * _H * _D // _PIECE
_HEAD_PAIRS = _S * _D // _PIECE
_WO_HEADS = _H // _NB
_HEADS_START = _W_PAIRS + _LAG + 4 * _H * _STAGE_PAIRS
_AHEAD = (_HEADS_START - 3 * _W_PAIRS) // _HEAD_PAIRS
_NSLOT = 3
assert _G * _HEAD_PAIRS + _LAG <= _AHEAD * _HEAD_PAIRS and _AHEAD <= 2 * _G

_WQ, _WUK, _WUV, _RING = 0, _NB, 2 * _NB, 3 * _NB
_CKV, _AWO, _BWO, _SPARE = 0, _B * _NB, (_B + 1) * _NB, (_B + 2) * _NB

_F32 = jnp.float32
_BF16 = jnp.bfloat16
_NT = (((1,), (1,)), ((), ()))


def _dot(a, b):
    return jnp.dot(a, b, preferred_element_type=_F32)


def _dot_nt(a, b):
    return lax.dot_general(a, b, _NT, preferred_element_type=_F32)


def _iota(shape, dim):
    return lax.broadcasted_iota(jnp.int32, shape, dim)


def _ds(index, size):
    start = index * size
    return pl.ds(start if isinstance(start, int) else pl.multiple_of(start, size), size)


def _wait_filled(dst, sem):
    pltpu.make_async_copy(dst, dst, sem).wait()


def _same_head_mask():
    shape = (_NB * _BH, 128)
    return (_iota(shape, 0) & (_H - 1)) == (_iota(shape, 1) & (_H - 1))


def _stack_columns(x):
    return jnp.concatenate([x[:, a * 128:(a + 1) * 128] for a in range(_NB)], axis=0)


def _contract_step(j, acc, lhs, w_rows, issue):
    src_minus_cl = _iota((128, 128), 0) - (_iota((128, 128), 1) >> 5)
    spread = jnp.where(src_minus_cl == 4 * j, 1.0, 0.0).astype(_BF16)
    e = jnp.where(_same_head_mask(), _dot(lhs, spread), 0.0).astype(_BF16)
    for a in range(_NB):
        acc = acc + _dot(e[a * _BH:(a + 1) * _BH], w_rows(a, j))
        issue(a, _NB)
    return acc


def _project_step(j, acc, q, w_rows, issue):
    t = []
    for a in range(_NB):
        t.append(_dot_nt(q, w_rows(a, j)))
        issue(a, _NB)
    t = jnp.where(_same_head_mask(), jnp.concatenate(t, axis=0), 0.0).astype(_BF16)
    dst_minus_cl = _iota((128, 128), 1) - (_iota((128, 128), 0) >> 5)
    gather = jnp.where(dst_minus_cl == 4 * j, 1.0, 0.0).astype(_BF16)
    return acc + _dot(t, gather)


def _kernel(ax_hbm, ckv_hbm, awq_hbm, awuk_hbm, awuv_hbm, awo_hbm,
            bx_hbm, k_hbm, v_hbm, bwq_hbm, bwo_hbm,
            out_ref,
            ax_v, bx_v, bwq_v, narrow_v, wide_v, qb_s, ob_s, ctx_s, s_s, sems):
    scale = _D ** -0.5

    def start_rows(src, buf, block, sem, n, priority):
        rows = _ds(n, _PIECE // _NB // src.shape[-1])
        pltpu.make_async_copy(src.at[:, rows], buf.at[pl.ds(block, _NB), rows],
                              sems.at[sem]).start(priority=priority)

    def start_queries(n):
        cols = _PIECE // _NB // 16
        per_row = _H * _D // cols
        piece = (slice(None), _ds(n // per_row, 16), _ds(n % per_row, cols))
        pltpu.make_async_copy(bwq_hbm.at[piece], bwq_v.at[piece], sems.at[0]).start(priority=0)
        start_rows(awq_hbm, narrow_v, _WQ, 2, n, 1)

    def start_up_projections(n):
        start_rows(awuk_hbm, narrow_v, _WUK, 1, n, 0)
        start_rows(awuv_hbm, narrow_v, _WUV, 1, n, 1)

    def start_latents(n):
        start_rows(ckv_hbm.at[0], wide_v, _CKV, 0, n, 0)
        start_rows(ckv_hbm.at[1], wide_v, _CKV + _NB, 0, n, 1)

    def ring_block(group, is_v):
        return _RING + ((group % _NSLOT) * 2 + is_v) * _G

    def start_kv(n):
        group = n // (_G * _HEAD_PAIRS)
        rows = _ds(n % (_G * _HEAD_PAIRS), _PIECE // _G // _D)
        for is_v, src in enumerate((k_hbm, v_hbm)):
            pltpu.make_async_copy(
                src.at[_ds(group, _G), rows],
                narrow_v.at[pl.ds(ring_block(group, is_v), _G), rows],
                sems.at[(group + 1) % 2]).start(priority=is_v)

    b_early_sem = (_BH // _G + 1) % 2

    def start_out_projections(n):
        t = n // (_W_PAIRS // _WO_HEADS)
        start_rows(awo_hbm, wide_v, _AWO, jnp.where(t < _EARLY, 2, 3), n, 0)
        start_rows(bwo_hbm, wide_v, _BWO,
                   jnp.where(t < _EARLY, b_early_sem, t - _EARLY + 4), n, 1)

    stream = ((_W_PAIRS, start_queries),
              (_W_PAIRS, start_up_projections),
              (_W_PAIRS, start_latents),
              (_BH * _HEAD_PAIRS, start_kv),
              (_W_PAIRS, start_out_projections))
    started = [0]

    def streaming_loop(lo, hi, pairs, body, carry, unroll=1):
        while lo < hi:
            first = started[0]
            for length, start in stream:
                if first < length:
                    break
                first -= length
            steps = min(hi - lo, (length - first) // pairs)
            assert steps > 0

            def step(j, carry, lo=lo, first=first, start=start):
                def issue(g, n):
                    for k in range(g * pairs // n, (g + 1) * pairs // n):
                        start(first + (j - lo) * pairs + k)
                return body(j, carry, issue)

            carry = lax.fori_loop(lo, lo + steps, step, carry, unroll=unroll)
            started[0] += steps * pairs
            lo += steps
        return carry

    def start_pairs(count):
        streaming_loop(0, count, 1, lambda j, carry, issue: issue(0, 1), None, unroll=4)

    def narrow_rows(block):
        return lambda a, j: narrow_v[block + a, _ds(j, 128), :]

    cp_bx = pltpu.make_async_copy(bx_hbm, bx_v, sems.at[3])
    cp_ax = pltpu.make_async_copy(ax_hbm, ax_v, sems.at[4])
    cp_bx.start()
    cp_ax.start()
    start_pairs(_W_PAIRS + _LAG - _LAG // 4)

    cp_bx.wait()
    _wait_filled(bwq_v, sems.at[0])
    qb = _dot(bx_v[...], bwq_v[...].reshape(_M, _H * _D))
    for h in range(_H):
        qb_s[pl.ds(h, _B, stride=_H), :] = qb[:, h * _D:(h + 1) * _D]
    start_pairs(_LAG // 4)

    def per_head_contract(lhs, block):
        lhs = _stack_columns(lhs).astype(_BF16)
        return streaming_loop(
            0, _H, _STAGE_PAIRS,
            lambda j, acc, issue: _contract_step(j, acc, lhs, narrow_rows(block), issue),
            jnp.zeros((_BH, _D), _F32))

    cp_ax.wait()
    _wait_filled(narrow_v.at[pl.ds(_WQ, _NB)], sems.at[2])
    x = ax_v[...].astype(_F32)
    x_rows = jnp.concatenate(
        [jnp.broadcast_to(x[b:b + 1], (_H, _M)) for b in range(_B)], axis=0)
    q = per_head_contract(x_rows, _WQ).astype(_BF16)

    _wait_filled(narrow_v.at[pl.ds(_WUK, 2 * _NB)], sems.at[1])
    qa = streaming_loop(
        0, _H, _STAGE_PAIRS,
        lambda j, acc, issue: _project_step(j, acc, q, narrow_rows(_WUK), issue),
        jnp.zeros((_NB * _BH, 128), _F32))

    _wait_filled(wide_v.at[pl.ds(_CKV, _B * _NB)], sems.at[0])
    steps_per_block = _S // _NB // _KC
    parts = _KC // 128
    latents = []
    for b in range(_B):
        qa_b = jnp.concatenate(
            [qa[a * _BH + b * _H:a * _BH + (b + 1) * _H] for a in range(_NB)],
            axis=1).astype(_BF16)

        def keys(c, part, b=b):
            return wide_v[_CKV + b * _NB + c // steps_per_block,
                          _ds((c % steps_per_block) * parts + part, 128), :]

        def scores(c, m, issue, qa_b=qa_b, keys=keys):
            s = []
            for part in range(parts):
                s.append(_dot_nt(qa_b, keys(c, part)))
                issue(part, parts)
            s = jnp.concatenate(s, axis=1) * scale
            s_s[c] = s
            return jnp.maximum(m, s)

        m = streaming_loop(0, _S // _KC, _STAGE_PAIRS, scores,
                           jnp.full((_H, _KC), -jnp.inf, _F32))
        m = jnp.max(m, axis=1, keepdims=True)

        def values(c, carry, issue, m=m, keys=keys):
            l, acc = carry
            p = jnp.exp(s_s[c] - m)
            l = l + p
            p = p.astype(_BF16)
            for part in range(parts):
                acc = acc + _dot(p[:, part * 128:(part + 1) * 128], keys(c, part))
                issue(part, parts)
            return l, acc

        l, acc = streaming_loop(0, _S // _KC, _STAGE_PAIRS, values,
                                (jnp.zeros((_H, _KC), _F32), jnp.zeros((_H, _M), _F32)))
        latents.append(acc / jnp.sum(l, axis=1, keepdims=True))

    ctx_s[...] = per_head_contract(jnp.concatenate(latents, axis=0), _WUV)

    def head(i, carry, issue, before_issue=lambda value: None):
        group, member = i // _G, i % _G
        k_block, v_block = ring_block(group, 0), ring_block(group, 1)
        kc = _S // _NC

        @pl.when(member == 0)
        def _():
            _wait_filled(narrow_v.at[pl.ds(k_block, 2 * _G)], sems.at[(group + 1) % 2])

        q = jnp.broadcast_to(qb_s[pl.ds(i, 1), :], (16, _D)).astype(_BF16)
        s = []
        for c in range(_NC):
            s.append(_dot_nt(q, narrow_v[k_block + member, _ds(c, kc), :]))
            before_issue(s[-1])
            issue(c, 2 * _NC)
        s = jnp.concatenate([part[:8] for part in s], axis=1) * scale
        p = jnp.exp(s - jnp.max(s, axis=1, keepdims=True))
        l = jnp.sum(p, axis=1, keepdims=True)
        p = jnp.concatenate([p, p], axis=0).astype(_BF16)
        o = jnp.zeros((16, _D), _F32)
        for c in range(_NC):
            part = _dot(p[:, c * kc:(c + 1) * kc], narrow_v[v_block + member, _ds(c, kc), :])
            before_issue(part)
            issue(_NC + c, 2 * _NC)
            o = o + part
        ob_s[pl.ds(i, 1), :] = (o[:8] / l)[0:1]
        return carry

    assert started[0] == _HEADS_START
    streaming_loop(0, _BH - _AHEAD, _HEAD_PAIRS, head, None)

    def last_head(i, carry, issue):
        def hold_back(value):
            wide_v[_SPARE, :16, :128] = value[:, :128].astype(_BF16)
        return head(i, carry, issue, hold_back)

    few, extra = divmod(_W_PAIRS, _AHEAD)
    streaming_loop(_BH - _AHEAD, _BH - _AHEAD + extra, few + 1, last_head, None)
    streaming_loop(_BH - _AHEAD + extra, _BH, few, last_head, None)
    assert started[0] == sum(length for length, _ in stream)

    def out_proj(ctx_ref, block, first, count, sem):
        _wait_filled(wide_v.at[pl.ds(block, _NB), pl.ds(first * _D, count * _D)], sems.at[sem])
        acc = jnp.zeros((_B, _M), _F32)
        for t in range(first, first + count):
            for a in range(_NB):
                ctx = ctx_ref[pl.ds(a * _WO_HEADS + t, _B, stride=_H), :]
                acc = acc + _dot(ctx.astype(_BF16), wide_v[block + a, _ds(t, _D), :])
        return acc

    out_a = out_proj(ctx_s, _AWO, 0, _EARLY, 2)
    out_b = out_proj(ob_s, _BWO, 0, _EARLY, b_early_sem)
    out_a = out_a + out_proj(ctx_s, _AWO, _EARLY, _WO_HEADS - _EARLY, 3)
    out_ref[:, :_M] = out_a.astype(out_ref.dtype)
    for t in range(_EARLY, _WO_HEADS):
        out_b = out_b + out_proj(ob_s, _BWO, t, 1, t - _EARLY + 4)
    out_ref[:, _M:] = out_b.astype(out_ref.dtype)


@jax.jit
def pallas_concat_heads__compressed_kv_cla__gqa_block_cached__decode_kernel(
    A_x: jax.Array,
    A_c_kv: jax.Array,
    A_w_q: jax.Array,
    A_w_uk: jax.Array,
    A_w_uv: jax.Array,
    A_w_o: jax.Array,
    B_x: jax.Array,
    B_k_cache: jax.Array,
    B_v_cache: jax.Array,
    B_wq: jax.Array,
    B_wo: jax.Array,
):
    assert A_x.shape == (_B, 1, _M) and B_x.shape == (_B, 1, _M)
    assert A_c_kv.shape == (_B, _S, _M)
    assert A_w_q.shape == A_w_uk.shape == A_w_uv.shape == (_M, _H, _D)
    assert A_w_o.shape == (_H, _D, _M)
    assert B_k_cache.shape == B_v_cache.shape == (_B, _H, _S, _D)
    assert B_wq.shape == (_M, _H * _D) and B_wo.shape == (_H * _D, _M)

    narrow = (_NB, _M * _H // _NB, _D)
    wide = (_NB, _H * _D // _NB, _M)
    vmem = pltpu.VMEM
    out = pl.pallas_call(
        _kernel,
        in_specs=[pl.BlockSpec(memory_space=pltpu.HBM)] * 11,
        out_specs=pl.BlockSpec(memory_space=vmem),
        out_shape=jax.ShapeDtypeStruct((_B, 2 * _M), A_x.dtype),
        scratch_shapes=[
            vmem((_B, _M), _BF16),
            vmem((_B, _M), _BF16),
            vmem((_NB, _M // _NB, _H * _D), _BF16),
            vmem((_RING + _NSLOT * 2 * _G,) + narrow[1:], _BF16),
            vmem((_SPARE + 1,) + wide[1:], _BF16),
            vmem((_BH, _D), _F32),
            vmem((_BH, _D), _F32),
            vmem((_BH, _D), _F32),
            vmem((_S // _KC, _H, _KC), _F32),
            pltpu.SemaphoreType.DMA((4 + _WO_HEADS - _EARLY,)),
        ],
        compiler_params=pltpu.CompilerParams(vmem_limit_bytes=100 * 2**20),
    )(
        A_x.reshape(_B, _M),
        A_c_kv.reshape((_B,) + wide),
        A_w_q.reshape(narrow),
        A_w_uk.reshape(narrow),
        A_w_uv.reshape(narrow),
        A_w_o.reshape(wide),
        B_x.reshape(_B, _M),
        B_k_cache.reshape(_BH, _S, _D),
        B_v_cache.reshape(_BH, _S, _D),
        B_wq.reshape(_NB, _M // _NB, _H * _D),
        B_wo.reshape(wide),
    )
    return out.reshape(_B, 1, 2 * _M)
```
